```python
import jax
import jax.numpy as jnp

def _softmax(x, axis=-1):
    return jax.nn.softmax(x, axis=axis)
def _gelu(x):
    return jax.nn.gelu(x, approximate=True)
def _silu(x):
    return jax.nn.silu(x)
def _sigmoid(x):
    return jax.nn.sigmoid(x)
def _layernorm(x, axis=-1, eps=1e-5):
    m = jnp.mean(x, axis=axis, keepdims=True)
    v = jnp.var(x, axis=axis, keepdims=True)
    return (x - m) / jnp.sqrt(v + eps)
def _scatter_add(tgt, idx, src, axis=0):
    return tgt.at[idx].add(src)
def _segment_sum(src, seg, n):
    return jax.ops.segment_sum(src, seg, n)
class _Rng:
    def __init__(self, key):
        self._k = key
    def _next(self):
        self._k, sub = jax.random.split(self._k)
        return sub
    def normal(self, shape):
        return jax.random.normal(self._next(), shape, dtype=jnp.bfloat16)
    def randint(self, lo, hi, shape):
        return jax.random.randint(self._next(), shape, lo, hi, dtype=jnp.int32)
    def uniform(self, shape, lo=0.0, hi=1.0):
        return jax.random.uniform(self._next(), shape, jnp.bfloat16, lo, hi)
    def permutation(self, n):
        return jax.random.permutation(self._next(), n)


kernel_name = 'recurrent_scan__sliding_block_cached__moe_arch_mod__decode'

def setup_inputs():
    _rng = _Rng(jax.random.key(int.from_bytes(__import__("os").urandom(4), "little")))
    _w = (lambda a: (lambda t: t.astype(jnp.bfloat16) if jnp.issubdtype(t.dtype, jnp.floating) else t)(jnp.asarray(a)))
    def _A_setup():
        B, Sq, D = 1, 1, 512
        Hq, Hkv, Sk, Dh = 32, 32, 32768, 128
        assert Hq % Hkv == 0, (Hq, Hkv)
        return {
            "x": _w((lambda *s: _rng.normal(s) * 0.05)(B, Sq, D)),
            "k_cache": _w((lambda *s: _rng.normal(s) * 0.05)(B, Hkv, Sk, Dh)),
            "v_cache": _w((lambda *s: _rng.normal(s) * 0.05)(B, Hkv, Sk, Dh)),
            "wq": _w((lambda *s: _rng.normal(s) * 0.05)(D, Hq * Dh) * (D ** -0.5)),
            "wo": _w((lambda *s: _rng.normal(s) * 0.05)(Hq * Dh, D) * ((Hq * Dh) ** -0.5)),
        }
    _A_in = _A_setup()

    def _B_setup():
        B, S, D, F, C = 1, 1, 512, 1376, 1
        return {
            "x": _w((lambda *s: _rng.normal(s) * 0.05)(B, S, D)),
            "w_r": _w((lambda *s: _rng.normal(s) * 0.05)(D)),
            "w_gate": _w((lambda *s: _rng.normal(s) * 0.05)(D, F)),
            "w_up": _w((lambda *s: _rng.normal(s) * 0.05)(D, F)),
            "w_down": _w((lambda *s: _rng.normal(s) * 0.05)(F, D)),
        }
    _B_in = _B_setup()

    return {
        "A_x": _A_in["x"],
        "A_k_cache": _A_in["k_cache"],
        "A_v_cache": _A_in["v_cache"],
        "A_wq": _A_in["wq"],
        "A_wo": _A_in["wo"],
        "B_x": _B_in["x"],
        "B_w_r": _B_in["w_r"],
        "B_w_gate": _B_in["w_gate"],
        "B_w_up": _B_in["w_up"],
        "B_w_down": _B_in["w_down"],
    }

def reference(A_x, A_k_cache, A_v_cache, A_wq, A_wo, B_x, B_w_r, B_w_gate, B_w_up, B_w_down):
    def _A_ref(x, k_cache, v_cache, wq, wo):
        B, Sq, D = x.shape
        Hq, Dh = 32, 128
        Hkv, Sk = k_cache.shape[1], k_cache.shape[2]
        W = min(4096, max(256, Sk // 4))
        rep = Hq // Hkv
        q = (lambda x, *d: x.transpose(*d))((x @ wq).reshape(B, Sq, Hq, Dh), 0, 2, 1, 3)
        k = jnp.repeat(k_cache[:, :, Sk - W:, :], rep, axis=1)
        v = jnp.repeat(v_cache[:, :, Sk - W:, :], rep, axis=1)
        scores = jnp.einsum("bhqd,bhkd->bhqk", q, k) * (Dh ** -0.5)
        p = _softmax(scores, axis=-1)
        o = jnp.einsum("bhqk,bhkd->bhqd", p, v)
        return (lambda x, *d: x.transpose(*d))(o, 0, 2, 1, 3).reshape(B, Sq, Hq * Dh) @ wo

    def _B_ref(x, w_r, w_gate, w_up, w_down):
        B, S, D = x.shape
        C = 1
        r = x @ w_r
        idx = jnp.argsort(-r, axis=-1)[:, :C]
        idx_e = jnp.repeat(idx.reshape(B, C, 1), D, axis=2)
        x_sel = jnp.take_along_axis(x, idx_e, axis=1)
        g = _silu(x_sel @ w_gate)
        u = x_sel @ w_up
        y = (g * u) @ w_down
        r_sel = _sigmoid(jnp.take_along_axis(r, idx, axis=1))
        y = y * r_sel.reshape(B, C, 1)
        b_off = (jnp.arange(B) * S).reshape(B, 1)
        flat_idx = (idx + b_off).reshape(B * C)
        zero = (x * 0.0).reshape(B * S, D)
        upd = _scatter_add(zero, flat_idx, y.reshape(B * C, D), axis=0)
        return x + upd.reshape(B, S, D)

    x = A_x
    xn = _layernorm(x, axis=-1)
    s = _A_ref(xn, A_k_cache, A_v_cache, A_wq, A_wo)
    g = _silu(_B_ref(xn, B_w_r, B_w_gate, B_w_up, B_w_down))
    return x + s * g
```

```python
import jax
import jax.numpy as jnp
import jax.experimental.pallas as pl
import jax.experimental.pallas.tpu as pltpu

D = 512
NH = 32
DH = 128
SK = 32768
W = min(4096, max(256, SK // 4))
F = 1376

CK = 128
NC = W // CK
NS = 2 * NC
PR = 32
FT = F // 32
FP = -(-F // 128)
RING = 8
LAG = 6
F0 = NS + LAG + 1
HEAD = (4, 7)
T_A = 1
T_0, T_E, T_O = 300, 110, 1
O_AT = {1: 6, 2: 3, 5: 7, 6: 4}
NAME = None
SCOPES = False

BF16 = jnp.bfloat16
F32 = jnp.float32
_NT = (((1,), (1,)), ((), ()))


def _div(n, d):
    return n // d if isinstance(n, int) else jax.lax.shift_right_logical(n, d.bit_length() - 1)


def _mod(n, d):
    return n & (d - 1)


def _ds(i, n):
    return pl.ds(i * n if isinstance(i, int) else pl.multiple_of(i * n, n), n)


def _pick(s, table):
    r = -1
    for k, v in table.items():
        r = jnp.where(s == k, v, r)
    return r


def _kernel(x_h, k_h, v_h, wq_h, wo_h, wr_h, wg_h, wu_h, wd_h, out_ref,
            x_v, wr_v, wq_v, kv_v, wo_v, wf_v, xn_v, q_v, s_v, m_v, l_v, o_v, h_v, y_v, c_v,
            s_x, s_q, s_kv, s_f, s_o):
    row = jax.lax.broadcasted_iota(jnp.int32, (8, DH), 0)
    row_d = jax.lax.broadcasted_iota(jnp.int32, (8, D), 0)

    def loop(name, n, body):
        if SCOPES:
            def body2(i, c):
                with jax.named_scope('y' + name):
                    return body(i, c)
            with jax.named_scope(name):
                jax.lax.fori_loop(0, n, body2, 0)
        else:
            jax.lax.fori_loop(0, n, body, 0)

    def wait_all(buf, sem):
        pltpu.make_async_copy(buf, buf, sem).wait()

    def copy_wq(j, t):
        rows, cols = _ds(t, 8), _ds(j, 512)
        return pltpu.make_async_copy(wq_h.at[:, rows, cols], wq_v.at[j, :, rows, :], s_q.at[j])

    def copy_kv(a, n, g, t):
        heads = pl.ds(_div(n, NC) * 16 + 4 * g, 4)
        r = pl.multiple_of(_mod(n, NC) * CK + t * PR, PR)
        return pltpu.make_async_copy((k_h, v_h)[a].at[0, heads, pl.ds(SK - W + r, PR), :],
                                     kv_v.at[a, heads, pl.ds(r, PR), :], s_kv.at[_mod(n, RING)])

    def copy_f(a, t):
        return pltpu.make_async_copy((wg_h, wu_h, wd_h)[a].at[:, pl.ds(pl.multiple_of(t * 16, 16), 16), :],
                                     wf_v.at[a, t], s_f.at[0])

    def copy_wo(u, t, sem):
        rows = pl.ds(pl.multiple_of(t * 8, 8), 8)
        return pltpu.make_async_copy(wo_h.at[_div(u, 4), :, _mod(u, 4), rows, :], wo_v.at[u, :, rows, :], sem)

    def q_proj(j, half):
        w = wq_v[j, :, :, pl.ds(half * 256, 256)].reshape(D, 256)
        q = jnp.dot(xn_v[...].astype(BF16), w, preferred_element_type=F32)
        for t in range(2):
            q_v[pl.ds(4 * j + 2 * half + t, 1), :] = q[0:1, t * DH:(t + 1) * DH]

    def qk(n, half):
        b, c = _div(n, NC) * 2 + half, _mod(n, NC)
        q = q_v[pl.ds(pl.multiple_of(b * 8, 8), 8), :].astype(BF16)
        keys = pl.ds(pl.multiple_of(c * CK, CK), CK)
        s = None
        for i in range(8):
            t = jax.lax.dot_general(q, kv_v[0, b * 8 + i, keys, :], _NT, preferred_element_type=F32)
            s = t if s is None else jnp.where(row == i, t, s)
        s = s * DH ** -0.5
        s_v[b, c] = s
        m_v[b] = jnp.maximum(m_v[b], s)

    def pv(n, half):
        b, c = _div(n, NC) * 2 + half, _mod(n, NC)
        p = jnp.exp(s_v[b, c] - m_v[b])
        l_v[b] += p
        p = p.astype(BF16)
        keys = pl.ds(pl.multiple_of(c * CK, CK), CK)
        o = None
        for i in range(8):
            t = jnp.dot(p, kv_v[1, b * 8 + i, keys, :], preferred_element_type=F32)
            o = t if o is None else jnp.where(row == i, t, o)
        o_v[b] += o

    def wait_kv(a, n):
        wait_all(kv_v.at[a, pl.ds(_div(n, NC) * 16, 16), pl.ds(pl.multiple_of(_mod(n, NC) * CK, CK), CK), :],
                 s_kv.at[_mod(n, RING)])

    def normalize(b):
        o_v[b] = o_v[b] / jnp.sum(l_v[b], axis=-1, keepdims=True)

    def ffn_rows(a, p):
        return wf_v[a, pl.ds(jnp.minimum(4 * p, FT - 4), 4)].reshape(128, D)

    def ffn_up(p):
        xn = xn_v[...].astype(BF16)
        g = jax.lax.dot_general(xn, ffn_rows(0, p), _NT, preferred_element_type=F32)
        u = jax.lax.dot_general(xn, ffn_rows(1, p), _NT, preferred_element_type=F32)
        lane = jax.lax.broadcasted_iota(jnp.int32, (8, 128), 1)
        h_v[...] = jnp.where(lane >= (p + 1) * 128 - F, jax.nn.silu(g) * u, 0.0)

    def ffn_down(p):
        y_v[0] += jnp.dot(h_v[...].astype(BF16), ffn_rows(2, p), preferred_element_type=F32)

    def o_proj(u, half):
        o = o_v[_div(u, 4) * 2 + half].astype(BF16)
        t0, t1 = [jnp.dot(o, wo_v[u, 2 * half + i], preferred_element_type=F32) for i in range(2)]
        y_v[1] += jnp.where(row_d == _mod(u, 4), t0, jnp.where(row_d == _mod(u, 4) + 4, t1, 0.0))

    copy_x = pltpu.make_async_copy(x_h, x_v, s_x.at[0])
    copy_wr = pltpu.make_async_copy(wr_h, wr_v, s_x.at[1])

    def next_wq(n, p):
        if p == 0:
            return copy_wq(_div(n, 8), _mod(n, 8))
        n0 = 64 - HEAD[0] * (HEAD[1] - 1) // 2
        if isinstance(n, int):
            return copy_wq(n // 8, 8 + n % 8)
        m = jnp.where(n < n0, 2 * n + 1, n + n0)
        return copy_wq(_div(m, 16), _div(_mod(m, 16), 2) + _mod(m, 2) * 8)

    for i in range(HEAD[0]):
        next_wq(i, 0).start(priority=0)
        for t in range(HEAD[1]):
            next_wq(i * HEAD[1] + t, 1).start(priority=1)
        if i == 0:
            copy_x.start()
            copy_wr.start()
        pl.delay(T_A)

    def head(i, carry):
        next_wq(HEAD[0] + i, 0).start(priority=0)
        next_wq(HEAD[0] * HEAD[1] + i, 1).start(priority=1)
        return carry

    loop('z_head', 64 - HEAD[0] * (HEAD[1] + 1) // 2, head)
    copy_f(2, FT - 1).start()
    m_v[...] = jnp.full(m_v.shape, -jnp.inf, F32)
    l_v[...] = jnp.zeros(l_v.shape, F32)
    o_v[...] = jnp.zeros(o_v.shape, F32)
    y_v[...] = jnp.zeros(y_v.shape, F32)

    copy_x.wait()
    copy_wr.wait()
    x = x_v[0].astype(F32)
    mean = jnp.mean(x, axis=-1, keepdims=True)
    var = jnp.mean(jnp.square(x - mean), axis=-1, keepdims=True)
    xn_v[...] = jnp.broadcast_to(((x - mean) / jnp.sqrt(var + 1e-5)).astype(BF16).astype(F32), (8, D))

    def halves(f):
        jax.lax.fori_loop(0, 2, lambda half, c: (f(half), c)[1], 0)

    def step(i, carry):
        n = i - LAG
        for a in range(2):
            @pl.when(_div(i, NS) == a)
            def _():
                def rows(t, c):
                    for g in range(4):
                        copy_kv(a, i - a * NS, g, t).start(priority=g % 2)
                    return c
                jax.lax.fori_loop(0, 4, rows, 0)

        @pl.when(i >= 2 * NS)
        def _():
            e = i - 2 * NS
            u0, r0 = 1 + _div(e, 2), _mod(e, 2) * 8
            u1, r1 = jnp.where(e < 4, 6 + _div(e, 2), jnp.where(e == 4, 5, 0)), jnp.where(e < 4, r0, 8)

            def rows(t, c):
                copy_wo(u0, r0 + t, s_o.at[u0]).start(priority=0)
                copy_wo(u1, r1 + t, s_o.at[jnp.where(e < 5, u1, 12 + _div(t, 2))]).start(priority=1)
                return c
            jax.lax.fori_loop(0, 8, rows, 0)

        @pl.when(i < FT)
        def _():
            copy_f(0, i).start(priority=0)
            copy_f(1, i).start(priority=1)

        @pl.when((i >= FT) & (i < FT + FT // 2))
        def _():
            copy_f(2, i - FT).start(priority=0)
            copy_f(2, i - FT + FT // 2).start(priority=1)

        @pl.when(i < 8)
        def _():
            wait_all(wq_v.at[i], s_q.at[i])
            q_proj(i, 0)
            q_proj(i, 1)

        @pl.when((n >= 0) & (n < NS))
        def _():
            wait_kv(0, n)
            halves(lambda half: qk(n, half))

        @pl.when(n >= NS)
        def _():
            wait_kv(1, n - NS)
            halves(lambda half: pv(n - NS, half))

        @pl.when(n == NS - 1)
        def _():
            for b in range(4):
                m_v[b] = jnp.broadcast_to(jnp.max(m_v[b], axis=-1, keepdims=True), (8, DH))

        @pl.when(i == F0 - 1)
        def _():
            wait_all(wf_v, s_f.at[0])

        @pl.when((i >= F0) & (i < F0 + FP))
        def _():
            ffn_up(i - F0)
            ffn_down(i - F0)

        @pl.when(i == F0 + FP)
        def _():
            xn = xn_v[...]
            r = jnp.sum(xn * wr_v[...].reshape(1, D).astype(F32), axis=-1, keepdims=True)
            y_v[0] = jax.nn.silu(xn + (xn * 0.0 + y_v[0] * jax.nn.sigmoid(r)))

        @pl.when((n >= NS) & (_mod(n, NC) == NC - 1))
        def _():
            normalize(_div(n - NS, NC) * 2)
            normalize(_div(n - NS, NC) * 2 + 1)

        @pl.when((n >= NS + NC) & (n < NS + NC + 4))
        def _():
            j = n - (NS + NC)
            o = o_v[_div(j, 2), pl.ds(_mod(j, 2) * 4, 1), :].astype(BF16).astype(F32)
            c_v[j] = jnp.broadcast_to(o, (DH, DH)).T
        return carry

    assert LAG == 6
    loop('z_step', 2 * NS + LAG, step)

    def tail(s, carry):
        e = s - 4
        u, half = _pick(_div(s, 2) - 2, {-2: 1, -1: 2, 8: 5, **O_AT}), _mod(s, 2)

        @pl.when(e == 0)
        def _():
            pl.delay(T_0)

        @pl.when((e >= 0) & (e < 16))
        def _():
            w = jnp.where(e < 12, 4 + _div(e, 8), 0)
            for t in range(2):
                copy_wo(w, 2 * jnp.where(e < 8, e, _mod(e, 4)) + t, s_o.at[jnp.where(e < 12, w, e - 4)]).start()

        @pl.when(u >= 0)
        def _():
            pl.when(half == 0)(lambda: wait_all(wo_v.at[u], s_o.at[u]))
            o_proj(u, half)

        @pl.when((u < 0) & (e < 15))
        def _():
            pl.delay(T_E)
        return carry

    loop('z_tail', 22, tail)

    part = y_v[1]
    gate = y_v[0]
    x = jnp.broadcast_to(x_v[0].astype(F32), (8, D))
    for i in (4, 0, 5, 1, 6, 2, 7, 3):
        rows = pl.ds(16 * i, 16)
        wait_all(wo_v.at[0, :, rows, :], s_o.at[8 + i])
        for j in range(4):
            prod = wo_v[0, j, rows, :].astype(F32) * jnp.concatenate([c_v[j, rows, :]] * (D // DH), axis=1)
            part = part + (prod[0:8] + prod[8:16])
    res = x + jnp.broadcast_to(jnp.sum(part, axis=0, keepdims=True), (8, D)) * gate
    out_ref[0] = res.astype(out_ref.dtype)[0:1]


def pallas_recurrent_scan__sliding_block_cached__moe_arch_mod__decode_kernel(
    A_x, A_k_cache, A_v_cache, A_wq, A_wo, B_x, B_w_r, B_w_gate, B_w_up, B_w_down,
):
    del B_x
    hbm = pl.BlockSpec(memory_space=pltpu.HBM)
    dma = pltpu.SemaphoreType.DMA
    return pl.pallas_call(
        lambda *refs: _kernel(*refs),
        name=NAME,
        out_shape=jax.ShapeDtypeStruct((1, 1, D), BF16),
        in_specs=[hbm] * 9,
        out_specs=pl.BlockSpec(memory_space=pltpu.VMEM),
        scratch_shapes=[
            pltpu.VMEM((1, 1, D), BF16),
            pltpu.VMEM((D,), BF16),
            pltpu.VMEM((8, 4, D // 4, 512), BF16),
            pltpu.VMEM((2, NH, W, DH), BF16),
            pltpu.VMEM((8, 4, DH, D), BF16),
            pltpu.VMEM((3, FT, 2, 16, D), BF16),
            pltpu.VMEM((8, D), F32),
            pltpu.VMEM((NH, DH), F32),
            pltpu.VMEM((4, NC, 8, CK), F32),
            pltpu.VMEM((4, 8, CK), F32),
            pltpu.VMEM((4, 8, CK), F32),
            pltpu.VMEM((4, 8, DH), F32),
            pltpu.VMEM((8, 128), F32),
            pltpu.VMEM((2, 8, D), F32),
            pltpu.VMEM((4, DH, DH), F32),
            dma((2,)), dma((8,)), dma((RING,)), dma((1,)), dma((16,)),
        ],
        compiler_params=pltpu.CompilerParams(
            vmem_limit_bytes=100 * 1024 * 1024,
            disable_semaphore_checks=True,
            disable_bounds_checks=True,
        ),
    )(A_x, A_k_cache, A_v_cache, A_wq.reshape(4, D // 4, NH * DH), A_wo.reshape(2, 4, 4, DH, D), B_w_r,
      B_w_gate.T.reshape(2, F // 2, D), B_w_up.T.reshape(2, F // 2, D), B_w_down.reshape(2, F // 2, D))
```

```python
import jax
import jax.numpy as jnp
import jax.experimental.pallas as pl
import jax.experimental.pallas.tpu as pltpu

D = 512
NH = 32
DH = 128
SK = 32768
W = min(4096, max(256, SK // 4))
F = 1376

CK = 256
NC = W // CK
NU = 4 * NC
KH = 9
FT = F // 16
FP = -(-F // 128)
RING = 32
LEAD = 3
LAG = 4
SKEW = 0
ROT = 37
PAD = 16
T_E = 120
TAIL = '0v 0o 0o 0v 0v 2- 1- 2v 2o 1o 2o 1o 1- 2o'
QUADS = (4, 5, 6, 7, 2, 1, 3)
VPU_ORDER = (0, 1, 2, 4, 5, 6, 3, 7)
NAME = None
SCOPES = False

BF16 = jnp.bfloat16
F32 = jnp.float32
_NT = (((1,), (1,)), ((), ()))


def _div(n, d):
    return n // d if isinstance(n, int) else jax.lax.shift_right_logical(n, d.bit_length() - 1)


def _mod(n, d):
    return n & (d - 1)


def _ds(i, n):
    return pl.ds(i * n if isinstance(i, int) else pl.multiple_of(i * n, n), n)


def _pick(s, table):
    word = [sum(v << 4 * j for j, v in enumerate(table[k:k + 8])) for k in (0, 8)]
    word = [w - (w >> 31 << 32) for w in word]
    return (jnp.where(s < 8, *word) >> 4 * _mod(s, 8)) & 15


def _kernel(x_h, k_h, v_h, wq_h, wo_h, wr_h, wg_h, wu_h, wd_h, out_ref,
            x_v, wr_v, wq_v, kv_v, wo_v, wf_v, xn_v, q_v, s_v, m_v, l_v, o_v, h_v, y_v, c_v,
            s_x, s_q, s_kv, s_f, s_o):
    row = jax.lax.broadcasted_iota(jnp.int32, (8, DH), 0)
    row_d = jax.lax.broadcasted_iota(jnp.int32, (8, D), 0)

    def loop(name, n, body):
        def body1(i, c):
            body(i)
            return c

        def body2(i, c):
            with jax.named_scope('y' + name):
                return body1(i, c)
        if SCOPES and name:
            with jax.named_scope(name):
                jax.lax.fori_loop(0, n, body2, 0)
        else:
            jax.lax.fori_loop(0, n, body1, 0)

    def wait_all(buf, sem):
        pltpu.make_async_copy(buf, buf, sem).wait()

    def sem_kv(a, u):
        if a == 0:
            return s_kv.at[jnp.where(u < NU - KH, _mod(u, RING), RING + u - (NU - KH))]
        return s_kv.at[_mod(NU - KH + u, RING)]

    def copy_kv(a, heads, odd, r, rows, sem):
        src = (SK - W) // rows + _mod(r + odd * (ROT * 64 // rows), W // rows)
        return pltpu.make_async_copy((k_h, v_h)[a].at[0, heads, _ds(src, rows), :],
                                     kv_v.at[a, heads, _ds(r, rows), :], sem)

    def copy_wo(u, heads, rows, sem):
        return pltpu.make_async_copy(wo_h.at[_div(u, 2), heads, _mod(u, 2), rows, :],
                                     wo_v.at[u, heads, rows, :], sem)

    def copy_f(a, r):
        return pltpu.make_async_copy((wg_h, wu_h, wd_h)[a].at[:, _ds(r, 8), :],
                                     wf_v.at[a, _div(r, 2), :, _ds(_mod(r, 2), 8), :], s_f.at[0])

    def lo_kv(a):
        def start(e, odd):
            u = _div(e, 4)
            r = _mod(u, NC) * 4 + _mod(e + odd * SKEW, 4)
            copy_kv(a, _ds(_div(u, NC) * 2 + odd, 4), odd, r, 64,
                    s_kv.at[_mod(a * (NU - KH) + u, RING)]).start(priority=1)
        return start

    def lo_wo(e, odd):
        vpu = e >= 8
        u = jnp.where(vpu, 0, 2 + _div(e, 4))
        r = jnp.where(vpu, e - 6, _mod(e, 4)) * 2 + odd
        copy_wo(u, slice(None), _ds(r, 16), s_o.at[jnp.where(vpu, 8 + r, u)]).start(priority=1)

    def hi_wq(e, odd):
        j, rows = _div(e, 16), _ds(_mod(e, 16), 8)
        pltpu.make_async_copy(wq_h.at[_ds(odd, 2), rows, _ds(j, 512)], wq_v.at[j, _ds(odd, 2), rows, :],
                              s_q.at[j]).start()

    def hi_k(e, odd):
        u = _div(e, 16)
        copy_kv(0, _ds(12 + _mod(_div(e, 8), 2) * 2 + odd, 2), _mod(_div(e, 8), 2), (NC - KH + u) * 8 + _mod(e, 8), 32,
                s_kv.at[RING + u]).start()

    def hi_f(e, odd):
        pl.when(e < FT)(lambda: copy_f(odd, e).start())
        pl.when(e >= FT)(lambda: copy_f(2, e - FT + odd * (FT // 2 - 1)).start())

    def hi_wo(e, odd):
        j, r = _div(e, 16), _mod(e, 16)
        u = jnp.where(j < 4, 4 + j, 5 - j)
        copy_wo(u, _ds(odd, 2), _ds(r, 8), s_o.at[jnp.where(u == 0, 8 + _div(r, 2), u)]).start()

    f0 = 32 + 4 * KH
    hi = [(0, hi_wq), (32, hi_k), (f0, hi_f), (f0 + 32, hi_wo)]
    lo = [(-LEAD, lo_kv(0)), (NU - KH - LEAD, lo_kv(1)), (2 * NU - KH - LEAD, lo_wo)]
    steps = lo[-1][0] + 3
    cuts = sorted({i for i, _ in hi + lo if i >= 0} | {steps})

    def q_proj(j, half):
        w = wq_v[j, :, :, _ds(half, 256)].reshape(D, 256)
        q = jnp.dot(xn_v[...].astype(BF16), w, preferred_element_type=F32)
        for t in range(2):
            q_v[pl.ds(4 * j + 2 * half + t, 1), :] = q[0:1, t * DH:(t + 1) * DH]

    def qk(b, keys):
        q = q_v[_ds(b, 8), :].astype(BF16)
        s = None
        for i in range(8):
            t = jax.lax.dot_general(q, kv_v[0, b * 8 + i, keys, :], _NT, preferred_element_type=F32)
            s = t if s is None else jnp.where(row_d[:, :CK] == i, t, s)
        s = s * DH ** -0.5
        s_v[b, :, keys] = s
        m_v[b] = jnp.maximum(m_v[b], s)

    def pv(b, keys):
        p = jnp.exp(s_v[b, :, keys] - m_v[b])
        l_v[b] += p
        p = p.astype(BF16)
        o = None
        for i in range(8):
            t = jnp.dot(p, kv_v[1, b * 8 + i, keys, :], preferred_element_type=F32)
            o = t if o is None else jnp.where(row == i, t, o)
        o_v[b] += o

    def attend(a, u):
        b, keys = _div(u, NC), _ds(_mod(u, NC), CK)
        wait_all(kv_v.at[a, _ds(b, 8), keys, :], sem_kv(a, u))
        (qk, pv)[a](b, keys)

        @pl.when(_mod(u, NC) == NC - 1)
        def _():
            if a == 0:
                m_v[b] = jnp.broadcast_to(jnp.max(m_v[b], axis=-1, keepdims=True), (8, CK))
            else:
                o_v[b] = o_v[b] / jnp.sum(l_v[b], axis=-1, keepdims=True)

    def ffn_rows(a, p):
        return wf_v[a, pl.ds(jnp.minimum(4 * p, FT // 2 - 4), 4)].reshape(128, D)

    def ffn_up(p):
        xn = xn_v[...].astype(BF16)
        g = jax.lax.dot_general(xn, ffn_rows(0, p), _NT, preferred_element_type=F32)
        u = jax.lax.dot_general(xn, ffn_rows(1, p), _NT, preferred_element_type=F32)
        lane = jax.lax.broadcasted_iota(jnp.int32, (8, 128), 1)
        h_v[...] = jnp.where(lane >= (p + 1) * 128 - F, jax.nn.silu(g) * u, 0.0)

    def ffn_down(p):
        y_v[0] += jnp.dot(h_v[...].astype(BF16), ffn_rows(2, p), preferred_element_type=F32)

    def o_proj(u):
        o = o_v[_div(u, 2)].astype(BF16)
        acc = 0.0
        for i in range(4):
            t = jnp.dot(o, wo_v[u, i], preferred_element_type=F32)
            acc = jnp.where(row_d == _mod(u, 2) + 2 * i, t, acc)
        y_v[1] += acc

    copy_x = pltpu.make_async_copy(x_h, x_v, s_x.at[0])
    copy_wr = pltpu.make_async_copy(wr_h, wr_v, s_x.at[1])
    for odd in range(2):
        lo_kv(0)(0, odd)
    copy_f(2, FT - 2).start()
    copy_x.start()
    copy_wr.start()
    loop(None, 4 * LEAD - 1, lambda e: [lo_kv(0)(e + 1, odd) for odd in range(2)])
    copy_f(2, FT - 1).start()
    m_v[...] = jnp.full(m_v.shape, -jnp.inf, F32)
    l_v[...] = jnp.zeros(l_v.shape, F32)
    o_v[...] = jnp.zeros(o_v.shape, F32)
    y_v[...] = jnp.zeros(y_v.shape, F32)

    def stream(i):
        for i0, i1 in zip(cuts, cuts[1:]):
            h0, start_hi = [e for e in hi if e[0] <= i0][-1]
            l0, start_lo = [e for e in lo if e[0] <= i0][-1]

            @pl.when((i >= i0) & (i < i1))
            def _():
                def pairs(t):
                    for odd in range(2):
                        start_hi((i - h0) * 4 + t, odd)
                        start_lo((i - l0) * 4 + t, odd)
                loop(None, 4 if i1 < steps else jnp.where(i < steps - 1, 4, 2), pairs)

        n = i - LAG

        @pl.when(i == LAG)
        def _():
            copy_x.wait()
            copy_wr.wait()
            x = x_v[0].astype(F32)
            mean = jnp.mean(x, axis=-1, keepdims=True)
            var = jnp.mean(jnp.square(x - mean), axis=-1, keepdims=True)
            xn_v[...] = jnp.broadcast_to(((x - mean) / jnp.sqrt(var + 1e-5)).astype(BF16).astype(F32), (8, D))

        @pl.when((n >= 3) & (n < 33) & (_mod(n + 1, 4) < 2))
        def _():
            j = _div(n - 3, 4)
            pl.when(_mod(n, 2) == 1)(lambda: wait_all(wq_v.at[j], s_q.at[j]))
            q_proj(j, _mod(n + 1, 2))

        pl.when((n >= 8) & (n < 8 + NU))(lambda: attend(0, n - 8))

        pl.when(n == f0 + 31)(lambda: wait_all(wf_v, s_f.at[0]))

        @pl.when((n >= f0 + 31) & (n < f0 + 31 + FP))
        def _():
            ffn_up(n - (f0 + 31))
            ffn_down(n - (f0 + 31))

        @pl.when(n == f0 + 31 + FP)
        def _():
            xn = xn_v[...]
            r = jnp.sum(xn * wr_v[...].reshape(1, D).astype(F32), axis=-1, keepdims=True)
            y_v[0] = jax.nn.silu(xn + (xn * 0.0 + y_v[0] * jax.nn.sigmoid(r)))

        @pl.when((n >= f0 + 26) & (n < f0 + 30))
        def _():
            j = n - (f0 + 26)
            o = o_v[0, pl.ds(2 * j, 1), :].astype(BF16).astype(F32)
            c_v[j] = jnp.broadcast_to(o, (DH, DH)).T

    tail = TAIL.split()
    e0, v0 = (steps - 1 - hi[-1][0]) * 4 + 2, steps - LAG - (NU - KH)
    first = [sum(int(t[0]) for t in tail[:j]) for j in range(len(tail) + 1)]
    chunks, quads = iter(range(8, 8 + NU - v0)), iter(QUADS)
    work = [next(chunks) if t[1] == 'v' else next(quads) if t[1] == 'o' else 0 for t in tail]
    assert e0 + first[-1] == 88 and e0 + first[work.index(1) + 1] >= 80 and not list(chunks) + list(quads)

    def step(i):
        pl.when(i < steps)(lambda: stream(i))
        s = i - steps
        w = jnp.where(s >= 0, _pick(s, work), -1)

        @pl.when(s >= 0)
        def _():
            e = _pick(s, first)
            loop(None, _pick(s + 1, first) - e, lambda t: [hi_wo(e0 + e + t, odd) for odd in range(2)])
            pl.when(w == 0)(lambda: pl.delay(T_E))

        e = i - (LAG + 8 + NU)
        loop(None, jnp.where(s >= 0, _div(w, 8), jnp.where(e < 0, 0, jnp.where(e < 8 + KH, 2, 1))),
             lambda j: attend(1, jnp.where(s >= 0, v0 + w - 8, jnp.where(e < 8 + KH, 2 * e + j, e + 8 + KH))))

        @pl.when((w > 0) & (w < 8))
        def _():
            wait_all(wo_v.at[w], s_o.at[w])
            o_proj(w)

    loop('z_step', steps + len(tail), step)

    part = y_v[1]
    gate = y_v[0]
    x = jnp.broadcast_to(x_v[0].astype(F32), (8, D))
    for i in VPU_ORDER:
        rows = pl.ds(16 * i, 16)
        wait_all(wo_v.at[0, :, rows, :], s_o.at[8 + i])
        for j in range(4):
            prod = wo_v[0, j, rows, :].astype(F32) * jnp.concatenate([c_v[j, rows, :]] * (D // DH), axis=1)
            part = part + (prod[0:8] + prod[8:16])
    res = x + jnp.broadcast_to(jnp.sum(part, axis=0, keepdims=True), (8, D)) * gate
    out_ref[0] = res.astype(out_ref.dtype)[0:1]


def pallas_recurrent_scan__sliding_block_cached__moe_arch_mod__decode_kernel(
    A_x, A_k_cache, A_v_cache, A_wq, A_wo, B_x, B_w_r, B_w_gate, B_w_up, B_w_down,
):
    del B_x
    hbm = pl.BlockSpec(memory_space=pltpu.HBM)
    dma = pltpu.SemaphoreType.DMA
    return pl.pallas_call(
        lambda *refs: _kernel(*refs),
        name=NAME,
        out_shape=jax.ShapeDtypeStruct((1, 1, D), BF16),
        in_specs=[hbm] * 9,
        out_specs=pl.BlockSpec(memory_space=pltpu.VMEM),
        scratch_shapes=[
            pltpu.VMEM((1, 1, D), BF16),
            pltpu.VMEM((D,), BF16),
            pltpu.VMEM((8, 4, D // 4, 512), BF16),
            pltpu.VMEM((2, NH, W + PAD, DH), BF16),
            pltpu.VMEM((8, 4, DH, D), BF16),
            pltpu.VMEM((3, FT // 2, 2, 16, D), BF16),
            pltpu.VMEM((8, D), F32),
            pltpu.VMEM((NH, DH), F32),
            pltpu.VMEM((4, 8, W), F32),
            pltpu.VMEM((4, 8, CK), F32),
            pltpu.VMEM((4, 8, CK), F32),
            pltpu.VMEM((4, 8, DH), F32),
            pltpu.VMEM((8, 128), F32),
            pltpu.VMEM((2, 8, D), F32),
            pltpu.VMEM((4, DH, DH), F32),
            dma((2,)), dma((8,)), dma((RING + KH,)), dma((1,)), dma((16,)),
        ],
        compiler_params=pltpu.CompilerParams(
            vmem_limit_bytes=100 * 1024 * 1024,
            disable_semaphore_checks=True,
            disable_bounds_checks=True,
        ),
    )(A_x, A_k_cache, A_v_cache, A_wq.reshape(4, D // 4, NH * DH), A_wo.reshape(4, 4, 2, DH, D), B_w_r,
      B_w_gate.T.reshape(2, F // 2, D), B_w_up.T.reshape(2, F // 2, D), B_w_down.reshape(2, F // 2, D))
```

```python
import jax
import jax.numpy as jnp
import jax.experimental.pallas as pl
import jax.experimental.pallas.tpu as pltpu

D = 512
NH = 32
DH = 128
SK = 32768
W = min(4096, max(256, SK // 4))
F = 1376

CK = 256
NC = W // CK
NU = 4 * NC
KH = 9
FT = F // 16
FP = -(-F // 128)
S18 = ''
QG = 2
LEAD = 3
LAG = 4
ROT = 37
PAD = 16
T_E = 120
TAIL = '0v 0v 0o 0o 0o 0v 2- 1- 2v 2o 1- 2o 1o 1- 2o'
QUADS = (0, 1, 2, 3, 6, 4, 7)
C0 = 56
VPU_ORDER = (0, 1, 2, 4, 5, 6, 3, 7)
NAME = None
SCOPES = False

BF16 = jnp.bfloat16
F32 = jnp.float32
_NT = (((1,), (1,)), ((), ()))


def _div(n, d):
    return n // d if isinstance(n, int) else jax.lax.shift_right_logical(n, d.bit_length() - 1)


def _mod(n, d):
    return n & (d - 1)


def _ds(i, n):
    return pl.ds(i * n if isinstance(i, int) else pl.multiple_of(i * n, n), n)


def _pick(s, table):
    word = [sum(v << 4 * j for j, v in enumerate(table[k:k + 8])) for k in (0, 8)]
    word = [w - (w >> 31 << 32) for w in word]
    return (jnp.where(s < 8, *word) >> 4 * _mod(s, 8)) & 15


def _kernel(x_h, k_h, v_h, wq_h, wo_h, wr_h, wg_h, wu_h, wd_h, out_ref,
            x_v, wr_v, wq_v, kv_v, wo_v, wf_v, xn_v, q_v, s_v, m_v, l_v, o_v, h_v, y_v, c_v,
            s_x, s_q, s_kv, s_f, s_o):
    row = jax.lax.broadcasted_iota(jnp.int32, (8, DH), 0)
    row_d = jax.lax.broadcasted_iota(jnp.int32, (8, D), 0)

    def loop(name, n, body):
        def body1(i, c):
            body(i)
            return c

        def body2(i, c):
            with jax.named_scope('y' + name):
                return body1(i, c)
        if SCOPES and name:
            with jax.named_scope(name):
                jax.lax.fori_loop(0, n, body2, 0)
        else:
            jax.lax.fori_loop(0, n, body1, 0)

    def wait_all(buf, sem):
        pltpu.make_async_copy(buf, buf, sem).wait()

    def copy_kv(a, heads, odd, r, rows, sem):
        src = (SK - W) // rows + _mod(r + odd * (ROT * 64 // rows), W // rows)
        return pltpu.make_async_copy((k_h, v_h)[a].at[0, heads, _ds(src, rows), :],
                                     kv_v.at[a, heads, _ds(r, rows), :], sem)

    def copy_wo(u, heads, rows, sem):
        return pltpu.make_async_copy(wo_h.at[heads, u, rows, :], wo_v.at[u, heads, rows, :], sem)

    def copy_f(a, r):
        if 'f' in S18:
            return pltpu.make_async_copy((wg_h, wu_h, wd_h)[a].at[_mod(r, 2), _ds(_div(r, 2), 16), :],
                                         wf_v.at[a, _div(r, 2), _mod(r, 2)], s_f.at[0])
        return pltpu.make_async_copy((wg_h, wu_h, wd_h)[a].at[:, _ds(r, 8), :],
                                     wf_v.at[a, _div(r, 2), :, _ds(_mod(r, 2), 8), :], s_f.at[0])

    def lo_kv(a):
        def start(e, odd):
            u = _div(e, 4)
            r = _mod(e, 4 * NC)
            copy_kv(a, _ds(_div(u, NC) * 2 + odd, 4), odd, r, 64,
                    s_kv.at[a * NU + u]).start(priority=1)
        return start

    def lo_wo(e, odd):
        vpu = e >= 8
        u = jnp.where(vpu, 5, 6 + _div(e, 4))
        r = jnp.where(vpu, e - 6, _mod(e, 4)) * 2 + odd
        copy_wo(u, slice(None), _ds(r, 16), s_o.at[jnp.where(vpu, 8 + r, u)]).start(priority=1)

    def hi_wq(e, odd):
        j = _div(e, 32)
        if 'q' in S18:
            a, rows, c = _mod(e, 2) * 2 + odd, _ds(_mod(_div(e, 2), 16), 8), slice(None)
            return pltpu.make_async_copy(wq_h.at[a, rows, _ds(j, 1024)], wq_v.at[j, a, rows, :], s_q.at[j]).start()
        if QG == 2:
            rows, c = _ds(_mod(_div(e, 2), 16), 8), _mod(e, 2)
        else:
            rows, c = _ds(_mod(e, 16), 8), _mod(_div(e, 16), 2)
        return pltpu.make_async_copy(wq_h.at[_ds(odd, 2), rows, _ds(2 * j + c, 512)],
                                     wq_v.at[j, _ds(odd, 2), rows, _ds(c, 512)], s_q.at[j]).start()

    def hi_k(e, odd):
        u = _div(e, 16)
        if 'k' in S18:
            g = _mod(_div(e, 8), 2)
            return copy_kv(0, 24 + 4 * g + _mod(e, 2) * 2 + odd, g, (NC - KH + u) * 4 + _mod(_div(e, 2), 4), 64,
                           s_kv.at[NU - KH + u]).start()
        copy_kv(0, _ds(12 + _mod(_div(e, 8), 2) * 2 + odd, 2), _mod(_div(e, 8), 2), (NC - KH + u) * 8 + _mod(e, 8), 32,
                s_kv.at[NU - KH + u]).start()

    def hi_f(e, odd):
        pl.when(e < FT)(lambda: copy_f(odd, e).start())
        pl.when(e >= FT)(lambda: copy_f(2, e - FT + odd * (FT // 2 - 1)).start())

    def hi_wo(e, odd):
        u, r = _div(e, 16), _mod(e, 16)
        heads, rows = (_mod(e, 2) * 2 + odd, _ds(_div(r, 2), 16)) if 'o' in S18 else (_ds(odd, 2), _ds(r, 8))
        copy_wo(u, heads, rows, s_o.at[jnp.where(u == 5, 8 + _div(r, 2), jnp.maximum(u, 3))]).start()

    f0 = 32 + 4 * KH
    q0 = 11
    hi = [(0, hi_wq), (32, hi_k), (f0, hi_f), (f0 + 32, hi_wo)]
    lo = [(-LEAD, lo_kv(0)), (NU - KH - LEAD, lo_kv(1)), (2 * NU - KH - LEAD, lo_wo)]
    steps = lo[-1][0] + 3
    cuts = sorted({i for i, _ in hi + lo if i >= 0} | {steps})

    def q_proj(j, half):
        w = wq_v[j, :, :, _ds(half, 256)].reshape(D, 256)
        q = jnp.dot(xn_v[...].astype(BF16), w, preferred_element_type=F32)
        for t in range(2):
            q_v[pl.ds(8 * j + 2 * half + t, 1), :] = q[0:1, t * DH:(t + 1) * DH]

    def qk(b, keys):
        q = q_v[_ds(b, 8), :].astype(BF16)
        s = None
        for i in range(8):
            t = jax.lax.dot_general(q, kv_v[0, b * 8 + i, keys, :], _NT, preferred_element_type=F32)
            s = t if s is None else jnp.where(row_d[:, :CK] == i, t, s)
        s = s * DH ** -0.5
        s_v[b, :, keys] = s
        m_v[b] = jnp.maximum(m_v[b], s)

    def pv(b, keys):
        p = jnp.exp(s_v[b, :, keys] - m_v[b])
        l_v[b] += p
        p = p.astype(BF16)
        o = None
        for i in range(8):
            t = jnp.dot(p, kv_v[1, b * 8 + i, keys, :], preferred_element_type=F32)
            o = t if o is None else jnp.where(row == i, t, o)
        o_v[b] += o

    def attend(a, u):
        b, keys = _div(u, NC), _ds(_mod(u, NC), CK)
        wait_all(kv_v.at[a, _ds(b, 8), keys, :], s_kv.at[a * NU + u])
        (qk, pv)[a](b, keys)

        @pl.when(_mod(u, NC) == NC - 1)
        def _():
            if a == 0:
                m_v[b] = jnp.broadcast_to(jnp.max(m_v[b], axis=-1, keepdims=True), (8, CK))
            else:
                o = o_v[b] / jnp.sum(l_v[b], axis=-1, keepdims=True)
                o_v[b] = o
                c_v[b] = jnp.broadcast_to(o[5:6].astype(BF16).astype(F32), (DH, DH)).T

    def ffn_rows(a, p):
        return wf_v[a, pl.ds(jnp.minimum(4 * p, FT // 2 - 4), 4)].reshape(128, D)

    def ffn_up(p):
        xn = xn_v[...].astype(BF16)
        g = jax.lax.dot_general(xn, ffn_rows(0, p), _NT, preferred_element_type=F32)
        u = jax.lax.dot_general(xn, ffn_rows(1, p), _NT, preferred_element_type=F32)
        lane = jax.lax.broadcasted_iota(jnp.int32, (8, 128), 1)
        h_v[...] = jnp.where(lane >= (p + 1) * 128 - F, jax.nn.silu(g) * u, 0.0)

    def ffn_down(p):
        y_v[0] += jnp.dot(h_v[...].astype(BF16), ffn_rows(2, p), preferred_element_type=F32)

    def o_proj(w):
        acc = y_v[1]
        for i in range(4):
            b, u = jnp.where(w < 4, w, i), jnp.where(w < 4, i, w)
            t = jnp.dot(o_v[b].astype(BF16), wo_v[u, b], preferred_element_type=F32)
            acc = acc + jnp.where(row_d == u, t, 0.0)
        y_v[1] = acc

    copy_x = pltpu.make_async_copy(x_h, x_v, s_x.at[0])
    copy_wr = pltpu.make_async_copy(wr_h, wr_v, s_x.at[1])
    for odd in range(2):
        lo_kv(0)(0, odd)
    copy_f(2, FT - 2).start()
    copy_x.start()
    copy_wr.start()
    loop(None, 4 * LEAD - 1, lambda e: [lo_kv(0)(e + 1, odd) for odd in range(2)])
    copy_f(2, FT - 1).start()
    m_v[...] = jnp.full(m_v.shape, -jnp.inf, F32)
    l_v[...] = jnp.zeros(l_v.shape, F32)
    o_v[...] = jnp.zeros(o_v.shape, F32)
    y_v[...] = jnp.zeros(y_v.shape, F32)

    def stream(i):
        for i0, i1 in zip(cuts, cuts[1:]):
            h0, start_hi = [e for e in hi if e[0] <= i0][-1]
            l0, start_lo = [e for e in lo if e[0] <= i0][-1]

            @pl.when((i >= i0) & (i < i1))
            def _():
                def pairs(t):
                    for odd in range(2):
                        start_hi((i - h0) * 4 + t, odd)
                        start_lo((i - l0) * 4 + t, odd)
                loop(None, 4 if i1 < steps else jnp.where(i < steps - 1, 4, 2), pairs)

        n = i - LAG

        @pl.when(i == LAG)
        def _():
            copy_x.wait()
            copy_wr.wait()
            x = x_v[0].astype(F32)
            mean = jnp.mean(x, axis=-1, keepdims=True)
            var = jnp.mean(jnp.square(x - mean), axis=-1, keepdims=True)
            xn_v[...] = jnp.broadcast_to(((x - mean) / jnp.sqrt(var + 1e-5)).astype(BF16).astype(F32), (8, D))

        e = n - (q0 - 4)
        @pl.when((e >= 0) & (e < 32) & (_mod(e, 8) < 4))
        def _():
            j = _div(e, 8)
            pl.when(_mod(e, 8) == 0)(lambda: wait_all(wq_v.at[j], s_q.at[j]))
            q_proj(j, _mod(e, 8))

        pl.when(n == f0 + 31)(lambda: wait_all(wf_v, s_f.at[0]))

        @pl.when((n >= f0 + 31) & (n < f0 + 31 + FP))
        def _():
            ffn_up(n - (f0 + 31))
            ffn_down(n - (f0 + 31))

        @pl.when(n == f0 + 31 + FP)
        def _():
            xn = xn_v[...]
            r = jnp.sum(xn * wr_v[...].reshape(1, D).astype(F32), axis=-1, keepdims=True)
            y_v[0] = jax.nn.silu(xn + (xn * 0.0 + y_v[0] * jax.nn.sigmoid(r)))

    tail = TAIL.split()
    e0, v0 = (steps - 1 - hi[-1][0]) * 4 + 2, steps - LAG - (NU - KH)
    first = [sum(int(t[0]) for t in tail[:j]) for j in range(len(tail) + 1)]
    chunks, quads = iter(range(8, 8 + NU - v0)), iter(QUADS)
    work = [next(chunks) if t[1] == 'v' else next(quads) if t[1] == 'o' else 15 for t in tail]
    assert e0 + first[-1] == 88 and e0 + first[work.index(4) + 1] >= 80 and not list(chunks) + list(quads)

    def step(i):
        pl.when(i < steps)(lambda: stream(i))
        s = i - steps
        w = jnp.where(s >= 0, _pick(s, work), -1)

        @pl.when(s >= 0)
        def _():
            e = _pick(s, first)
            loop(None, _pick(s + 1, first) - e, lambda t: [hi_wo(e0 + e + t, odd) for odd in range(2)])
            pl.when(w == 15)(lambda: pl.delay(T_E))

        e = i - (LAG + q0)
        late = q0 + KH
        done = e + jnp.clip(e - C0, 0, late)

        def chunk(j):
            u = jnp.where(s >= 0, NU + v0 + w - 8, done + j)
            for a in range(2):
                pl.when(_div(u, NU) == a)(lambda: attend(a, u - a * NU))

        loop(None, jnp.where(s >= 0, ((w >= 8) & (w < 15)).astype(jnp.int32),
                             jnp.where(e < 0, 0, jnp.where((e >= C0) & (e < C0 + late), 2, 1))), chunk)

        @pl.when((w >= 0) & (w < 8))
        def _():
            pl.when(w == 0)(lambda: wait_all(wo_v.at[pl.ds(0, 4)], s_o.at[3]))
            pl.when(w >= 4)(lambda: wait_all(wo_v.at[w], s_o.at[w]))
            o_proj(w)

    assert C0 + 2 * q0 + KH + LAG <= steps
    loop('z_step', steps + len(tail), step)

    part = y_v[1]
    gate = y_v[0]
    x = jnp.broadcast_to(x_v[0].astype(F32), (8, D))
    for i in VPU_ORDER:
        rows = pl.ds(16 * i, 16)
        wait_all(wo_v.at[5, :, rows, :], s_o.at[8 + i])
        for j in range(4):
            prod = wo_v[5, j, rows, :].astype(F32) * jnp.concatenate([c_v[j, rows, :]] * (D // DH), axis=1)
            part = part + (prod[0:8] + prod[8:16])
    res = x + jnp.broadcast_to(jnp.sum(part, axis=0, keepdims=True), (8, D)) * gate
    out_ref[0] = res.astype(out_ref.dtype)[0:1]


def pallas_recurrent_scan__sliding_block_cached__moe_arch_mod__decode_kernel(
    A_x, A_k_cache, A_v_cache, A_wq, A_wo, B_x, B_w_r, B_w_gate, B_w_up, B_w_down,
):
    del B_x
    hbm = pl.BlockSpec(memory_space=pltpu.HBM)
    dma = pltpu.SemaphoreType.DMA
    return pl.pallas_call(
        lambda *refs: _kernel(*refs),
        name=NAME,
        out_shape=jax.ShapeDtypeStruct((1, 1, D), BF16),
        in_specs=[hbm] * 9,
        out_specs=pl.BlockSpec(memory_space=pltpu.VMEM),
        scratch_shapes=[
            pltpu.VMEM((1, 1, D), BF16),
            pltpu.VMEM((D,), BF16),
            pltpu.VMEM((4, 4, D // 4, 1024), BF16),
            pltpu.VMEM((2, NH, W + PAD, DH), BF16),
            pltpu.VMEM((8, 4, DH, D), BF16),
            pltpu.VMEM((3, FT // 2, 2, 16, D), BF16),
            pltpu.VMEM((8, D), F32),
            pltpu.VMEM((NH, DH), F32),
            pltpu.VMEM((4, 8, W), F32),
            pltpu.VMEM((4, 8, CK), F32),
            pltpu.VMEM((4, 8, CK), F32),
            pltpu.VMEM((4, 8, DH), F32),
            pltpu.VMEM((8, 128), F32),
            pltpu.VMEM((2, 8, D), F32),
            pltpu.VMEM((4, DH, DH), F32),
            dma((2,)), dma((8,)), dma((2 * NU,)), dma((1,)), dma((16,)),
        ],
        compiler_params=pltpu.CompilerParams(
            vmem_limit_bytes=100 * 1024 * 1024,
            disable_semaphore_checks=True,
            disable_bounds_checks=True,
        ),
    )(A_x, A_k_cache, A_v_cache, A_wq.reshape(4, D // 4, NH * DH), A_wo.reshape(4, 8, DH, D), B_w_r,
      B_w_gate.T.reshape(2, F // 2, D), B_w_up.T.reshape(2, F // 2, D), B_w_down.reshape(2, F // 2, D))
```

```python
import jax
import jax.numpy as jnp
import jax.experimental.pallas as pl
import jax.experimental.pallas.tpu as pltpu

D = 512
NH = 32
DH = 128
SK = 32768
W = min(4096, max(256, SK // 4))
F = 1376

CK = 256
NC = W // CK
NU = 4 * NC
VH = 9
SHIFT = 1
FT = F // 16
FP = -(-F // 128)
LEAD = 3
LAG = 4
Q0 = 19
C0 = 50
TAIL = "0v 0v 0o 0o 0o 0v 2- 1- 2v 2o 1- 2o 1o 1- 2o"
QUADS = (5, 6, 7, 1, 3, 2, 4)
T_IDLE = 120
VPU_ORDER = (0, 1, 2, 4, 5, 6, 3, 7)
SCOPES = False

BF16 = jnp.bfloat16
F32 = jnp.float32
_NT = (((1,), (1,)), ((), ()))


def _div(n, d):
    return n // d if isinstance(n, int) else jax.lax.shift_right_logical(n, d.bit_length() - 1)


def _mod(n, d):
    return n & (d - 1)


def _ds(i, n):
    return pl.ds(i * n if isinstance(i, int) else pl.multiple_of(i * n, n), n)


def _swap(h):
    return (h & 19) | ((h & 4) << 1) | ((h & 8) >> 1)


def _v_slot(h):
    return _swap(_mod(h + NH - SHIFT, NH))


def _pick(s, table):
    word = [sum(v << 4 * j for j, v in enumerate(table[k:k + 8])) for k in (0, 8)]
    word = [w - (w >> 31 << 32) for w in word]
    return (jnp.where(s < 8, *word) >> 4 * _mod(s, 8)) & 15


def _loop(n, body):
    def body1(i, carry):
        body(i)
        return carry
    jax.lax.fori_loop(0, n, body1, 0)


def _kernel(x_h, k_h, v_h, wq_h, wo_h, wr_h, wg_h, wu_h, wd_h, out_ref,
            x_v, wr_v, wq_v, kv_v, wo_v, wf_v, xn_v, q_v, s_v, m_v, l_v, o_v, y_v, c_v,
            s_x, s_q, s_kv, s_f, s_o):
    def wait_all(buf, sem):
        pltpu.make_async_copy(buf, buf, sem).wait()

    def copy_kv(a, head, slot, n, r):
        return pltpu.make_async_copy((k_h, v_h)[a].at[0, pl.ds(head, n), _ds((SK - W) // 64 + r, 64), :],
                                     kv_v.at[a, pl.ds(slot, n), _ds(r, 64), :],
                                     s_kv.at[a * NU + _div(slot, 8) * NC + _div(r, 4)])

    def copy_wo(u, heads, rows, sem):
        return pltpu.make_async_copy(wo_h.at[heads, u, rows, :], wo_v.at[u, heads, rows, :], sem)

    def copy_f(a, r):
        return pltpu.make_async_copy((wg_h, wu_h, wd_h)[a].at[:, _ds(r, 8), :],
                                     wf_v.at[a, _div(r, 2), :, _ds(_mod(r, 2), 8), :], s_f.at[0])

    def lo_k(e, odd):
        slot = _div(e, 64) * 8 + 4 * odd
        copy_kv(0, _swap(slot), slot, 4, _mod(e, 64)).start(priority=1)

    def lo_v(e, odd):
        n = 4 * (NC - VH)
        slot = jnp.where(e < n, 24, _div(e - n, 64) * 8 + 4 * odd)
        copy_kv(1, _swap(slot) + SHIFT, slot, 4, jnp.where(e < n, e + odd * n, _mod(e - n, 64))).start(priority=1)

    def lo_wo(e, odd):
        vpu = e >= 8
        u = jnp.where(vpu, 0, 3 + _div(e, 4))
        r = jnp.where(vpu, e - 6, _mod(e, 4)) * 2 + odd
        copy_wo(u, slice(None), _ds(r, 16), s_o.at[jnp.where(vpu, 8 + r, u)]).start(priority=1)

    def hi_wq(e, odd):
        j, rows, c = _div(e, 32), _ds(_mod(_div(e, 2), 16), 8), _mod(e, 2)
        pltpu.make_async_copy(wq_h.at[_ds(odd, 2), rows, _ds(2 * j + c, 512)],
                              wq_v.at[j, _ds(odd, 2), rows, _ds(c, 512)], s_q.at[j]).start()

    def hi_v(e, odd):
        slot = jnp.where(e < 128, 28, 24) + _mod(e, 2) * 2 + odd
        r = _div(e, 2) - jnp.where(e < 128, 0, 8 * VH - 64)
        copy_kv(1, _mod(_swap(slot) + SHIFT, NH), slot, 1, r).start()

    def hi_f(e, odd):
        pl.when(e < FT)(lambda: copy_f(odd, e).start())
        pl.when(e >= FT)(lambda: copy_f(2, e - FT + odd * (FT // 2 - 1)).start())

    def hi_wo(e, odd):
        u, r = _pick(_div(e, 16), (5, 6, 7, 1, 2, 0)), _mod(e, 16)
        copy_wo(u, _ds(odd, 2), _ds(r, 8), s_o.at[jnp.where(u == 0, 8 + _div(r, 2), u)]).start()

    f0 = 32 + 4 * VH
    hi = [(0, hi_wq), (32, hi_v), (f0, hi_f), (f0 + 32, hi_wo)]
    lo = [(-LEAD, lo_k), (NU - LEAD, lo_v), (2 * NU - VH - LEAD, lo_wo)]
    steps = lo[-1][0] + 3
    cuts = sorted({i for i, _ in hi + lo if i >= 0} | {steps})

    def head_row(ref, r):
        return jnp.broadcast_to(ref[pl.ds(r, 1), :], (8, DH)).astype(BF16)

    def q_proj(j):
        w = wq_v[_div(j, 4), :, :, _ds(_mod(j, 4), 256)].reshape(D, 256)
        q = jnp.dot(xn_v[...].astype(BF16), w, preferred_element_type=F32)
        for t in range(2):
            q_v[pl.ds(2 * j + t, 1), :] = q[0:1, t * DH:(t + 1) * DH]

    def qk(b, c):
        for i in range(8):
            h = _swap(8 * b + i)
            s = jax.lax.dot_general(head_row(q_v, h), kv_v[0, 8 * b + i, _ds(c, CK), :], _NT,
                                    preferred_element_type=F32) * DH ** -0.5
            for j in range(CK // 128):
                s_v[c, j, pl.ds(_v_slot(h), 1), :] = s[0:1, j * 128:(j + 1) * 128]

    def pv(b, c):
        rows = _ds(b, 8)
        p = [jnp.exp(s_v[c, j, rows, :] - m_v[rows, :]) for j in range(CK // 128)]
        l_v[rows, :] += sum(p)
        p = jnp.concatenate(p, axis=1).astype(BF16)
        row = jax.lax.broadcasted_iota(jnp.int32, (8, DH), 0)
        o = None
        for i in range(8):
            t = jnp.dot(p, kv_v[1, 8 * b + i, _ds(c, CK), :], preferred_element_type=F32)
            o = t if o is None else jnp.where(row == i, t, o)
        o_v[rows, :] += o

        @pl.when(c == NC - 1)
        def _():
            o_v[rows, :] = o_v[rows, :] / jnp.sum(l_v[rows, :], axis=-1, keepdims=True)

    def attend(a, u):
        b, c = _mod(_div(u, NC) + 3 * a, 4), _mod(u, NC)
        wait_all(kv_v.at[a, _ds(b, 8), _ds(c, CK), :], s_kv.at[a * NU + b * NC + c])
        (qk, pv)[a](b, c)

        if a == 0:
            @pl.when(u == NU - 1)
            def _():
                m = jax.lax.fori_loop(0, NC, lambda c, m: jnp.maximum(m, jnp.max(s_v[c], axis=0)),
                                      jnp.full((NH, 128), -jnp.inf, F32))
                m_v[...] = jnp.broadcast_to(jnp.max(m, axis=-1, keepdims=True), (NH, 128))

    def ffn(p):
        wg, wu, wd = [wf_v[a, pl.ds(jnp.minimum(4 * p, FT // 2 - 4), 4)].reshape(128, D) for a in range(3)]
        xn = xn_v[...].astype(BF16)
        g = jax.lax.dot_general(xn, wg, _NT, preferred_element_type=F32)
        u = jax.lax.dot_general(xn, wu, _NT, preferred_element_type=F32)
        lane = jax.lax.broadcasted_iota(jnp.int32, (8, 128), 1)
        hid = jnp.where(lane >= (p + 1) * 128 - F, jax.nn.silu(g) * u, 0.0)
        y_v[0] += jnp.dot(hid.astype(BF16), wd, preferred_element_type=F32)

    def o_proj(u):
        y_v[1] += sum(jnp.dot(head_row(o_v, _v_slot(u + 8 * i)), wo_v[u, i], preferred_element_type=F32)
                      for i in range(4))

    copy_x = pltpu.make_async_copy(x_h, x_v, s_x.at[0])
    copy_wr = pltpu.make_async_copy(wr_h, wr_v, s_x.at[1])
    for odd in range(2):
        lo_k(0, odd)
    copy_f(2, FT - 2).start()
    copy_x.start()
    copy_wr.start()
    _loop(4 * LEAD - 1, lambda e: [lo_k(e + 1, odd) for odd in range(2)])
    copy_f(2, FT - 1).start()
    l_v[...] = jnp.zeros(l_v.shape, F32)
    o_v[...] = jnp.zeros(o_v.shape, F32)
    y_v[...] = jnp.zeros(y_v.shape, F32)

    def stream(i):
        for i0, i1 in zip(cuts, cuts[1:]):
            h0, start_hi = [e for e in hi if e[0] <= i0][-1]
            l0, start_lo = [e for e in lo if e[0] <= i0][-1]

            @pl.when((i >= i0) & (i < i1))
            def _():
                def pairs(t):
                    for odd in range(2):
                        start_hi((i - h0) * 4 + t, odd)
                        start_lo((i - l0) * 4 + t, odd)
                _loop(4 if i1 < steps else jnp.where(i < steps - 1, 4, 2), pairs)

        n = i - LAG

        @pl.when(n == 0)
        def _():
            copy_x.wait()
            copy_wr.wait()
            x = x_v[0].astype(F32)
            mean = jnp.mean(x, axis=-1, keepdims=True)
            var = jnp.mean(jnp.square(x - mean), axis=-1, keepdims=True)
            xn_v[...] = jnp.broadcast_to(((x - mean) / jnp.sqrt(var + 1e-5)).astype(BF16).astype(F32), (8, D))

        @pl.when((n >= 7) & (n < 39) & (_mod(n - 7, 8) < 4))
        def _():
            j = _div(n - 7, 8)
            pl.when(_mod(n - 7, 8) == 0)(lambda: wait_all(wq_v.at[j], s_q.at[j]))
            q_proj(4 * j + _mod(n - 7, 8))

        pl.when(n == f0 + 31)(lambda: wait_all(wf_v, s_f.at[0]))
        pl.when((n >= f0 + 31) & (n < f0 + 31 + FP))(lambda: ffn(n - (f0 + 31)))

        @pl.when(n == f0 + 31 + FP)
        def _():
            xn = xn_v[...]
            r = jnp.sum(xn * wr_v[...].reshape(1, D).astype(F32), axis=-1, keepdims=True)
            y_v[0] = jax.nn.silu(xn + (xn * 0.0 + y_v[0] * jax.nn.sigmoid(r)))

        @pl.when(i >= steps - 4)
        def _():
            j = i - (steps - 4)
            c_v[j] = jnp.broadcast_to(head_row(o_v, _v_slot(8 * j)).astype(F32)[0:1], (DH, DH)).T

    tail = TAIL.split()
    e0, v0 = (steps - 1 - hi[-1][0]) * 4 + 2, NU - (LEAD + LAG - 3)
    first = [sum(int(t[0]) for t in tail[:j]) for j in range(len(tail) + 1)]
    chunks, quads = iter(range(8, 8 + NU - v0)), iter(QUADS)
    work = [next(chunks) if t[1] == "v" else next(quads) if t[1] == "o" else 0 for t in tail]
    late = Q0 + VH
    assert e0 + first[-1] == 88 and e0 + first[work.index(2) + 1] >= 80 and not list(chunks) + list(quads)
    assert steps - LAG - Q0 + late == NU + v0 and LAG + Q0 + C0 + late <= steps - 4

    def step(i):
        pl.when(i < steps)(lambda: stream(i))
        s = i - steps
        w = jnp.where(s >= 0, _pick(s, work), 0)

        @pl.when(s >= 0)
        def _():
            e = _pick(s, first)
            _loop(_pick(s + 1, first) - e, lambda t: [hi_wo(e0 + e + t, odd) for odd in range(2)])
            pl.when(w == 0)(lambda: pl.delay(T_IDLE))

        e = i - (LAG + Q0)
        done = jnp.where(s >= 0, NU + v0 + w - 8, e + jnp.clip(e - C0, 0, late))

        def chunk(j):
            for a in range(2):
                pl.when(_div(done + j, NU) == a)(lambda: attend(a, done + j - a * NU))

        _loop(jnp.where(s >= 0, _div(w, 8), jnp.where(e < 0, 0, jnp.where((e >= C0) & (e < C0 + late), 2, 1))),
              chunk)

        @pl.when((w > 0) & (w < 8))
        def _():
            wait_all(wo_v.at[w], s_o.at[w])
            o_proj(w)

    def scoped(i):
        with jax.named_scope('yz_step'):
            step(i)

    _loop(steps + len(tail), scoped if SCOPES else step)

    part = jnp.where(jax.lax.broadcasted_iota(jnp.int32, (8, D), 0) == 0, y_v[1], 0.0)
    gate = y_v[0]
    x = jnp.broadcast_to(x_v[0].astype(F32), (8, D))
    for i in VPU_ORDER:
        rows = _ds(i, 16)
        wait_all(wo_v.at[0, :, rows, :], s_o.at[8 + i])
        for j in range(4):
            prod = wo_v[0, j, rows, :].astype(F32) * jnp.concatenate([c_v[j, rows, :]] * (D // DH), axis=1)
            part = part + (prod[0:8] + prod[8:16])
    res = x + jnp.broadcast_to(jnp.sum(part, axis=0, keepdims=True), (8, D)) * gate
    out_ref[0] = res.astype(out_ref.dtype)[0:1]


@jax.jit
def pallas_recurrent_scan__sliding_block_cached__moe_arch_mod__decode_kernel(
    A_x: jax.Array,
    A_k_cache: jax.Array,
    A_v_cache: jax.Array,
    A_wq: jax.Array,
    A_wo: jax.Array,
    B_x: jax.Array,
    B_w_r: jax.Array,
    B_w_gate: jax.Array,
    B_w_up: jax.Array,
    B_w_down: jax.Array,
):
    del B_x
    hbm = pl.BlockSpec(memory_space=pltpu.HBM)
    dma = pltpu.SemaphoreType.DMA
    return pl.pallas_call(
        _kernel,
        out_shape=jax.ShapeDtypeStruct((1, 1, D), BF16),
        in_specs=[hbm] * 9,
        out_specs=pl.BlockSpec(memory_space=pltpu.VMEM),
        scratch_shapes=[
            pltpu.VMEM((1, 1, D), BF16),
            pltpu.VMEM((D,), BF16),
            pltpu.VMEM((4, 4, D // 4, 1024), BF16),
            pltpu.VMEM((2, NH, W + 16, DH), BF16),
            pltpu.VMEM((8, 4, DH, D), BF16),
            pltpu.VMEM((3, FT // 2, 2, 16, D), BF16),
            pltpu.VMEM((8, D), F32),
            pltpu.VMEM((NH, DH), F32),
            pltpu.VMEM((NC, CK // 128, NH, 128), F32),
            pltpu.VMEM((NH, 128), F32),
            pltpu.VMEM((NH, 128), F32),
            pltpu.VMEM((NH, DH), F32),
            pltpu.VMEM((2, 8, D), F32),
            pltpu.VMEM((4, DH, DH), F32),
            dma((2,)), dma((4,)), dma((2 * NU,)), dma((1,)), dma((16,)),
        ],
        compiler_params=pltpu.CompilerParams(
            vmem_limit_bytes=100 * 1024 * 1024,
            disable_bounds_checks=True,
            disable_semaphore_checks=True,
        ),
    )(A_x, A_k_cache, A_v_cache, A_wq.reshape(4, D // 4, NH * DH), A_wo.reshape(4, 8, DH, D), B_w_r,
      B_w_gate.T.reshape(2, F // 2, D), B_w_up.T.reshape(2, F // 2, D), B_w_down.reshape(2, F // 2, D))
```

```python
import jax
import jax.numpy as jnp
import jax.experimental.pallas as pl
import jax.experimental.pallas.tpu as pltpu

D = 512
NH = 32
DH = 128
SK = 32768
W = min(4096, max(256, SK // 4))
F = 1376

CK = 256
NC = W // CK
NU = 4 * NC
VH = 9
SHIFT = 1
FT = F // 16
FP = -(-F // 128)
LEAD = 3
LAG = 4
Q0 = 23
C0, C1 = 16, 52
TAIL = "0v 0v 0o 0o 0o 0- 2v 1v 1- 2o 2- 2o 1o 1- 2o"
QUADS = (5, 6, 7, 1, 3, 2, 4)
T_IDLE = 70
VPU_ORDER = (0, 1, 2, 4, 5, 6, 3, 7)

BF16 = jnp.bfloat16
F32 = jnp.float32
_NT = (((1,), (1,)), ((), ()))


def _div(n, d):
    return n // d if isinstance(n, int) else jax.lax.shift_right_logical(n, d.bit_length() - 1)


def _mod(n, d):
    return n & (d - 1)


def _ds(i, n):
    return pl.ds(i * n if isinstance(i, int) else pl.multiple_of(i * n, n), n)


def _k_head(slot):
    return (slot & 19) | ((slot & 4) << 1) | ((slot & 8) >> 1)


def _v_head(slot):
    return _mod((((slot & 11) + _div(slot, 16) * 4) ^ ((slot & 4) * 6)) + SHIFT, NH)


def _v_slot(head):
    h = _mod(head + NH - SHIFT, NH)
    low = h ^ (_div(h, 16) * 24)
    return (low & 11) + (low & 4) * 4 + _div(h, 16) * 4


def _pick(s, table):
    word = [sum(v << 4 * j for j, v in enumerate(table[k:k + 8])) for k in (0, 8)]
    word = [w - (w >> 31 << 32) for w in word]
    return (jnp.where(s < 8, *word) >> 4 * _mod(s, 8)) & 15


def _loop(n, body):
    def body1(i, carry):
        body(i)
        return carry
    jax.lax.fori_loop(0, n, body1, 0)


def _kernel(x_h, k_h, v_h, wq_h, wo_h, wr_h, wg_h, wu_h, wd_h, out_ref,
            x_v, wr_v, wq_v, kv_v, wo_v, wf_v, xn_v, q_v, s_v, m_v, l_v, o_v, y_v, c_v,
            s_x, s_q, s_kv, s_f, s_o):
    def wait_all(buf, sem):
        pltpu.make_async_copy(buf, buf, sem).wait()

    def copy_kv(a, head, slot, n, r):
        return pltpu.make_async_copy((k_h, v_h)[a].at[0, pl.ds(head, n), _ds((SK - W) // 64 + r, 64), :],
                                     kv_v.at[a, pl.ds(slot, n), _ds(r, 64), :],
                                     s_kv.at[a * NU + _div(slot, 8) * NC + _div(r, 4)])

    def copy_wo(u, heads, rows, sem):
        return pltpu.make_async_copy(wo_h.at[heads, u, rows, :], wo_v.at[u, heads, rows, :], sem)

    def copy_f(a, r):
        return pltpu.make_async_copy((wg_h, wu_h, wd_h)[a].at[_mod(r, 2), _ds(_div(r, 2), 16), :],
                                     wf_v.at[a, _ds(r, 16), :], s_f.at[0])

    def lo_k(e, odd):
        slot = _div(e, 64) * 8 + 4 * odd
        copy_kv(0, _k_head(slot), slot, 4, _mod(e, 64)).start(priority=1)

    def lo_v2(e, odd):
        copy_kv(1, _v_head(16), 16, 4, e + odd * 4 * (NC - VH)).start(priority=1)

    def lo_v(e, odd):
        slot = _mod(_div(e, 64) + 3, 4) * 8 + 4 * odd
        copy_kv(1, _v_head(slot), slot, 4, _mod(e, 64)).start(priority=1)

    def lo_wo(e, odd):
        vpu = e >= 8
        u = jnp.where(vpu, 0, 3 + _div(e, 4))
        r = jnp.where(vpu, e - 6, _mod(e, 4)) * 2 + odd
        copy_wo(u, slice(None), _ds(r, 16), s_o.at[jnp.where(vpu, 8 + r, u)]).start(priority=1)

    def hi_wq(e, odd):
        j, a, rows = _div(e, 64) * 2 + _mod(_div(e, 2), 2), _mod(e, 2) * 2 + odd, _ds(_mod(_div(e, 4), 16), 8)
        pltpu.make_async_copy(wq_h.at[a, rows, _ds(j, 1024)], wq_v.at[j, a, rows, :], s_q.at[j]).start()

    def hi_v(e, odd):
        slot = jnp.where(e < 128, 20, 16) + _mod(e, 2) * 2 + odd
        r = _div(e, 2) - jnp.where(e < 128, 0, 8 * VH - 64)
        copy_kv(1, _v_head(slot), slot, 1, r).start()

    def hi_f(e, odd):
        r = _div((2 * e + odd) * 171, 512)
        for a in range(3):
            pl.when(2 * e + odd - 3 * r == a)(lambda: copy_f(a, r).start())

    def hi_wo(e, odd):
        u, r = _pick(_div(e, 16), (5, 6, 7, 1, 2, 0)), _mod(e, 16)
        copy_wo(u, _ds(odd, 2), _ds(r, 8), s_o.at[jnp.where(u == 0, 8 + _div(r, 2), u)]).start()

    f0 = 32 + 4 * VH
    hi = [(0, hi_wq), (32, hi_v), (f0, hi_f), (f0 + 32, hi_wo)]
    lo = [(-LEAD, lo_k), (NU - LEAD, lo_v2), (NU + NC - VH - LEAD, lo_v), (2 * NU - VH - LEAD, lo_wo)]
    steps = lo[-1][0] + 3
    cuts = sorted({i for i, _ in hi + lo if i >= 0} | {steps})

    def head_row(ref, r):
        return jnp.broadcast_to(ref[pl.ds(r, 1), :], (8, DH)).astype(BF16)

    def q_proj(j):
        w = wq_v[_div(j, 4), :, :, _ds(_mod(j, 4), 256)].reshape(D, 256)
        q = jnp.dot(xn_v[...].astype(BF16), w, preferred_element_type=F32)
        for t in range(2):
            q_v[pl.ds(2 * j + t, 1), :] = q[0:1, t * DH:(t + 1) * DH]

    def qk(b, c):
        for i in range(8):
            h = _k_head(8 * b + i)
            s = jax.lax.dot_general(head_row(q_v, h), kv_v[0, 8 * b + i, _ds(c, CK), :], _NT,
                                    preferred_element_type=F32) * DH ** -0.5
            for j in range(CK // 128):
                s_v[c, j, pl.ds(_v_slot(h), 1), :] = s[0:1, j * 128:(j + 1) * 128]

    def pv(b, c):
        rows = _ds(b, 8)
        p = [jnp.exp(s_v[c, j, rows, :] - m_v[rows, :]) for j in range(CK // 128)]
        l_v[rows, :] += sum(p)
        p = jnp.concatenate(p, axis=1).astype(BF16)
        row = jax.lax.broadcasted_iota(jnp.int32, (8, DH), 0)
        o = None
        for i in range(8):
            t = jnp.dot(p, kv_v[1, 8 * b + i, _ds(c, CK), :], preferred_element_type=F32)
            o = t if o is None else jnp.where(row == i, t, o)
        o_v[rows, :] += o

        @pl.when(c == NC - 1)
        def _():
            o_v[rows, :] = o_v[rows, :] / jnp.sum(l_v[rows, :], axis=-1, keepdims=True)

    def attend(a, u):
        b, c = _mod(_div(u, NC) + 2 * a, 4), _mod(u, NC)
        wait_all(kv_v.at[a, _ds(b, 8), _ds(c, CK), :], s_kv.at[a * NU + b * NC + c])
        (qk, pv)[a](b, c)

        if a == 0:
            @pl.when(u == NU - 1)
            def _():
                m = jax.lax.fori_loop(0, NC, lambda c, m: jnp.maximum(m, jnp.max(s_v[c], axis=0)),
                                      jnp.full((NH, 128), -jnp.inf, F32))
                m_v[...] = jnp.broadcast_to(jnp.max(m, axis=-1, keepdims=True), (NH, 128))

    def ffn(p):
        wg, wu, wd = [wf_v[a, pl.ds(pl.multiple_of(jnp.minimum(128 * p, F - 128), 16), 128), :] for a in range(3)]
        xn = xn_v[...].astype(BF16)
        g = jax.lax.dot_general(xn, wg, _NT, preferred_element_type=F32)
        u = jax.lax.dot_general(xn, wu, _NT, preferred_element_type=F32)
        lane = jax.lax.broadcasted_iota(jnp.int32, (8, 128), 1)
        hid = jnp.where(lane >= (p + 1) * 128 - F, jax.nn.silu(g) * u, 0.0)
        y_v[0] += jnp.dot(hid.astype(BF16), wd, preferred_element_type=F32)

    def o_proj(u):
        y_v[1] += sum(jnp.dot(head_row(o_v, _v_slot(u + 8 * i)), wo_v[u, i], preferred_element_type=F32)
                      for i in range(4))

    copy_x = pltpu.make_async_copy(x_h, x_v, s_x.at[0])
    copy_wr = pltpu.make_async_copy(wr_h, wr_v, s_x.at[1])
    for odd in range(2):
        lo_k(0, odd)
    copy_f(1, FT - 1).start()
    copy_x.start()
    copy_wr.start()
    _loop(4 * LEAD - 1, lambda e: [lo_k(e + 1, odd) for odd in range(2)])
    copy_f(2, FT - 1).start()
    l_v[...] = jnp.zeros(l_v.shape, F32)
    o_v[...] = jnp.zeros(o_v.shape, F32)
    y_v[...] = jnp.zeros(y_v.shape, F32)

    def stream(i):
        for i0, i1 in zip(cuts, cuts[1:]):
            h0, start_hi = [e for e in hi if e[0] <= i0][-1]
            l0, start_lo = [e for e in lo if e[0] <= i0][-1]

            @pl.when((i >= i0) & (i < i1))
            def _():
                def pairs(t):
                    for odd in range(2):
                        start_hi((i - h0) * 4 + t, odd)
                        start_lo((i - l0) * 4 + t, odd)
                _loop(4 if i1 < steps else jnp.where(i < steps - 1, 4, 2), pairs)

        n = i - LAG

        @pl.when(n == 0)
        def _():
            copy_x.wait()
            copy_wr.wait()
            x = x_v[0].astype(F32)
            mean = jnp.mean(x, axis=-1, keepdims=True)
            var = jnp.mean(jnp.square(x - mean), axis=-1, keepdims=True)
            xn_v[...] = jnp.broadcast_to(((x - mean) / jnp.sqrt(var + 1e-5)).astype(BF16).astype(F32), (8, D))

        @pl.when((n >= 15) & (n < 47) & (_mod(n - 15, 16) < 8))
        def _():
            j = _div(n - 15, 16) * 8 + _mod(n - 15, 8)
            pl.when(_mod(j, 4) == 0)(lambda: wait_all(wq_v.at[_div(j, 4)], s_q.at[_div(j, 4)]))
            q_proj(j)

        pl.when(n == f0 + 31)(lambda: wait_all(wf_v, s_f.at[0]))
        pl.when((n >= f0 + 31) & (n < f0 + 31 + FP))(lambda: ffn(n - (f0 + 31)))

        @pl.when(n == f0 + 31 + FP)
        def _():
            xn = xn_v[...]
            r = jnp.sum(xn * wr_v[...].reshape(1, D).astype(F32), axis=-1, keepdims=True)
            y_v[0] = jax.nn.silu(xn + (xn * 0.0 + y_v[0] * jax.nn.sigmoid(r)))

        @pl.when(i >= steps - 4)
        def _():
            j = i - (steps - 4)
            c_v[j] = jnp.broadcast_to(head_row(o_v, _v_slot(8 * j)).astype(F32)[0:1], (DH, DH)).T

    tail = TAIL.split()
    e0, v0 = (steps - 1 - hi[-1][0]) * 4 + 2, NU - (LEAD + LAG - 3)
    first = [sum(int(t[0]) for t in tail[:j]) for j in range(len(tail) + 1)]
    chunks, quads = iter(range(8, 8 + NU - v0)), iter(QUADS)
    work = [next(chunks) if t[1] == "v" else next(quads) if t[1] == "o" else 0 for t in tail]
    assert e0 + first[-1] == 88 and e0 + first[work.index(2) + 1] >= 80 and not list(chunks) + list(quads)
    assert steps - LAG + VH == NU + v0 and LAG + Q0 + C1 + VH <= steps - 4

    def step(i):
        pl.when(i < steps)(lambda: stream(i))
        s = i - steps
        w = jnp.where(s >= 0, _pick(s, work), 0)

        @pl.when(s >= 0)
        def _():
            e = _pick(s, first)
            _loop(_pick(s + 1, first) - e, lambda t: [hi_wo(e0 + e + t, odd) for odd in range(2)])
            pl.when(w == 0)(lambda: pl.delay(T_IDLE))

        e = i - (LAG + Q0)
        done = jnp.where(s >= 0, NU + v0 + w - 8, e + jnp.clip(e - C0, 0, Q0) + jnp.clip(e - C1, 0, VH))

        two = ((e >= C0) & (e < C0 + Q0)) | ((e >= C1) & (e < C1 + VH))

        def chunk(j):
            for a in range(2):
                pl.when(_div(done + j, NU) == a)(lambda: attend(a, done + j - a * NU))

        _loop(jnp.where(s >= 0, _div(w, 8), jnp.where(e < 0, 0, jnp.where(two, 2, 1))), chunk)

        @pl.when((w > 0) & (w < 8))
        def _():
            wait_all(wo_v.at[w], s_o.at[w])
            o_proj(w)

    _loop(steps + len(tail), step)

    part = jnp.where(jax.lax.broadcasted_iota(jnp.int32, (8, D), 0) == 0, y_v[1], 0.0)
    gate = y_v[0]
    x = jnp.broadcast_to(x_v[0].astype(F32), (8, D))
    for i in VPU_ORDER:
        rows = _ds(i, 16)
        wait_all(wo_v.at[0, :, rows, :], s_o.at[8 + i])
        for j in range(4):
            prod = wo_v[0, j, rows, :].astype(F32) * jnp.concatenate([c_v[j, rows, :]] * (D // DH), axis=1)
            part = part + (prod[0:8] + prod[8:16])
    res = x + jnp.broadcast_to(jnp.sum(part, axis=0, keepdims=True), (8, D)) * gate
    out_ref[0] = res.astype(out_ref.dtype)[0:1]


@jax.jit
def pallas_recurrent_scan__sliding_block_cached__moe_arch_mod__decode_kernel(
    A_x: jax.Array,
    A_k_cache: jax.Array,
    A_v_cache: jax.Array,
    A_wq: jax.Array,
    A_wo: jax.Array,
    B_x: jax.Array,
    B_w_r: jax.Array,
    B_w_gate: jax.Array,
    B_w_up: jax.Array,
    B_w_down: jax.Array,
):
    del B_x
    hbm = pl.BlockSpec(memory_space=pltpu.HBM)
    dma = pltpu.SemaphoreType.DMA
    return pl.pallas_call(
        _kernel,
        out_shape=jax.ShapeDtypeStruct((1, 1, D), BF16),
        in_specs=[hbm] * 9,
        out_specs=pl.BlockSpec(memory_space=pltpu.VMEM),
        scratch_shapes=[
            pltpu.VMEM((1, 1, D), BF16),
            pltpu.VMEM((D,), BF16),
            pltpu.VMEM((4, 4, D // 4, 1024), BF16),
            pltpu.VMEM((2, NH, W + 16, DH), BF16),
            pltpu.VMEM((8, 4, DH, D), BF16),
            pltpu.VMEM((3, F, D), BF16),
            pltpu.VMEM((8, D), F32),
            pltpu.VMEM((NH, DH), F32),
            pltpu.VMEM((NC, CK // 128, NH, 128), F32),
            pltpu.VMEM((NH, 128), F32),
            pltpu.VMEM((NH, 128), F32),
            pltpu.VMEM((NH, DH), F32),
            pltpu.VMEM((2, 8, D), F32),
            pltpu.VMEM((4, DH, DH), F32),
            dma((2,)), dma((4,)), dma((2 * NU,)), dma((1,)), dma((16,)),
        ],
        compiler_params=pltpu.CompilerParams(
            vmem_limit_bytes=100 * 1024 * 1024,
            disable_bounds_checks=True,
            disable_semaphore_checks=True,
        ),
    )(A_x, A_k_cache, A_v_cache, A_wq.reshape(4, D // 4, NH * DH), A_wo.reshape(4, 8, DH, D), B_w_r,
      B_w_gate.T.reshape(2, F // 2, D), B_w_up.T.reshape(2, F // 2, D), B_w_down.reshape(2, F // 2, D))
```

```python
import jax
import jax.numpy as jnp
import jax.experimental.pallas as pl
import jax.experimental.pallas.tpu as pltpu

D = 512
NH = 32
DH = 128
SK = 32768
W = min(4096, max(256, SK // 4))
F = 1376

CK = 256
NC = W // CK
NU = 4 * NC
VH = 9
SHIFT = 1
FT = F // 16
FP = -(-F // 128)
LEAD = 3
LAG = 4
Q0 = 23
C0, C1 = 16, 52
TAIL = "0v 0v 0o 0o 0o 0- 2v 1v 1- 2o 2- 2o 1o 1- 2o"
QUADS = (5, 6, 7, 1, 3, 2, 4)
T_IDLE = 70
VPU_ORDER = (0, 1, 4, 2, 5, 3, 6, 7)

BF16 = jnp.bfloat16
F32 = jnp.float32
_NT = (((1,), (1,)), ((), ()))


def _div(n, d):
    return n // d if isinstance(n, int) else jax.lax.shift_right_logical(n, d.bit_length() - 1)


def _mod(n, d):
    return n & (d - 1)


def _ds(i, n):
    return pl.ds(i * n if isinstance(i, int) else pl.multiple_of(i * n, n), n)


def _k_head(slot):
    return (_div(slot, 8) * 4 + _mod(slot, 4)) ^ ((slot & 4) * 6)


def _v_head(slot):
    return _mod((((slot & 11) + _div(slot, 16) * 4) ^ ((slot & 4) * 6)) + SHIFT, NH)


def _v_slot(head):
    h = _mod(head + NH - SHIFT, NH)
    low = h ^ (_div(h, 16) * 24)
    return (low & 11) + (low & 4) * 4 + _div(h, 16) * 4


def _pick(s, table):
    word = [sum(v << 4 * j for j, v in enumerate(table[k:k + 8])) for k in (0, 8)]
    word = [w - (w >> 31 << 32) for w in word]
    return (jnp.where(s < 8, *word) >> 4 * _mod(s, 8)) & 15


def _loop(n, body):
    def body1(i, carry):
        body(i)
        return carry
    jax.lax.fori_loop(0, n, body1, 0)


def _kernel(x_h, k_h, v_h, wq_h, wo_h, wr_h, wg_h, wu_h, wd_h, out_ref,
            x_v, wr_v, wq_v, kv_v, wo_v, wf_v, xn_v, q_v, s_v, m_v, l_v, o_v, y_v, c_v,
            s_x, s_q, s_kv, s_f, s_o):
    def wait_all(buf, sem):
        pltpu.make_async_copy(buf, buf, sem).wait()

    def copy_kv(a, head, slot, n, r):
        return pltpu.make_async_copy((k_h, v_h)[a].at[0, pl.ds(head, n), _ds((SK - W) // 64 + r, 64), :],
                                     kv_v.at[a, pl.ds(slot, n), _ds(r, 64), :],
                                     s_kv.at[a * NU + _div(slot, 8) * NC + _div(r, 4)])

    def copy_wo(u, heads, rows, sem):
        return pltpu.make_async_copy(wo_h.at[heads, u, rows, :], wo_v.at[u, heads, rows, :], sem)

    def copy_f(a, r):
        return pltpu.make_async_copy((wg_h, wu_h, wd_h)[a].at[_mod(r, 2), _ds(_div(r, 2), 16), :],
                                     wf_v.at[a, _ds(r, 16), :], s_f.at[0])

    def lo_k(e, odd):
        slot = _div(e, 128) * 16 + _mod(e, 2) * 8 + 4 * odd
        copy_kv(0, _k_head(slot), slot, 4, _mod(_div(e, 2), 64)).start(priority=1)

    def lo_v2(e, odd):
        copy_kv(1, _v_head(16), 16, 4, e + odd * 4 * (NC - VH)).start(priority=1)

    def lo_v(e, odd):
        slot = _mod(_div(e, 64) + 3, 4) * 8 + 4 * odd
        copy_kv(1, _v_head(slot), slot, 4, _mod(e, 64)).start(priority=1)

    def lo_wo(e, odd):
        vpu = e >= 8
        u = jnp.where(vpu, 0, 3 + _div(e, 4))
        r = jnp.where(vpu, e - 6, _mod(e, 4)) * 2 + odd
        copy_wo(u, slice(None), _ds(r, 16), s_o.at[jnp.where(vpu, 8 + r, u)]).start(priority=1)

    def hi_wq(e, odd):
        j, a, rows = _mod(_div(e, 64) * 2 + _mod(_div(e, 2), 2) + 3, 4), _mod(e, 2) * 2 + odd, _ds(_mod(_div(e, 4), 16), 8)
        pltpu.make_async_copy(wq_h.at[a, rows, _ds(j, 1024)], wq_v.at[j, a, rows, :], s_q.at[j]).start()

    def hi_v(e, odd):
        slot = jnp.where(e < 128, 20, 16) + _mod(e, 2) * 2 + odd
        r = _div(e, 2) - jnp.where(e < 128, 0, 8 * VH - 64)
        copy_kv(1, _v_head(slot), slot, 1, r).start()

    def hi_f(e, odd):
        r = _div((2 * e + odd) * 171, 512)
        for a in range(3):
            pl.when(2 * e + odd - 3 * r == a)(lambda: copy_f(a, r).start())

    def hi_wo(e, odd):
        u, r = _pick(_div(e, 16), (5, 6, 7, 1, 2, 0)), _mod(e, 16)
        copy_wo(u, _ds(odd, 2), _ds(r, 8), s_o.at[jnp.where(u == 0, 8 + _div(r, 2), u)]).start()

    f0 = 32 + 4 * VH
    hi = [(0, hi_wq), (32, hi_v), (f0, hi_f), (f0 + 32, hi_wo)]
    lo = [(-LEAD, lo_k), (NU - LEAD, lo_v2), (NU + NC - VH - LEAD, lo_v), (2 * NU - VH - LEAD, lo_wo)]
    steps = lo[-1][0] + 3
    cuts = sorted({i for i, _ in hi + lo if i >= 0} | {steps})

    def head_row(ref, r):
        return jnp.broadcast_to(ref[pl.ds(r, 1), :], (8, DH)).astype(BF16)

    def q_proj(j):
        w = wq_v[_div(j, 4), :, :, _ds(_mod(j, 4), 256)].reshape(D, 256)
        q = jnp.dot(xn_v[...].astype(BF16), w, preferred_element_type=F32)
        for t in range(2):
            q_v[pl.ds(2 * j + t, 1), :] = q[0:1, t * DH:(t + 1) * DH]

    def qk(b, c):
        for i in range(8):
            h = _k_head(8 * b + i)
            s = jax.lax.dot_general(head_row(q_v, h), kv_v[0, 8 * b + i, _ds(c, CK), :], _NT,
                                    preferred_element_type=F32) * DH ** -0.5
            for j in range(CK // 128):
                s_v[c, j, pl.ds(_v_slot(h), 1), :] = s[0:1, j * 128:(j + 1) * 128]

    def pv(b, c):
        rows = _ds(b, 8)
        p = [jnp.exp(s_v[c, j, rows, :] - m_v[rows, :]) for j in range(CK // 128)]
        l_v[rows, :] += sum(p)
        p = jnp.concatenate(p, axis=1).astype(BF16)
        row = jax.lax.broadcasted_iota(jnp.int32, (8, DH), 0)
        o = None
        for i in range(8):
            t = jnp.dot(p, kv_v[1, 8 * b + i, _ds(c, CK), :], preferred_element_type=F32)
            o = t if o is None else jnp.where(row == i, t, o)
        o_v[rows, :] += o

        @pl.when(c == NC - 1)
        def _():
            o_v[rows, :] = o_v[rows, :] / jnp.sum(l_v[rows, :], axis=-1, keepdims=True)

    def attend(a, u):
        b, c = (_mod(_div(u, NC) + 2, 4), _mod(u, NC)) if a else (_div(u, 2 * NC) * 2 + _mod(u, 2), _mod(_div(u, 2), NC))
        wait_all(kv_v.at[a, _ds(b, 8), _ds(c, CK), :], s_kv.at[a * NU + b * NC + c])
        (qk, pv)[a](b, c)

        if a == 0:
            @pl.when(u == NU - 1)
            def _():
                m = jax.lax.fori_loop(0, NC, lambda c, m: jnp.maximum(m, jnp.max(s_v[c], axis=0)),
                                      jnp.full((NH, 128), -jnp.inf, F32))
                m_v[...] = jnp.broadcast_to(jnp.max(m, axis=-1, keepdims=True), (NH, 128))

    def ffn(p):
        wg, wu, wd = [wf_v[a, pl.ds(pl.multiple_of(jnp.minimum(128 * p, F - 128), 16), 128), :] for a in range(3)]
        xn = xn_v[...].astype(BF16)
        g = jax.lax.dot_general(xn, wg, _NT, preferred_element_type=F32)
        u = jax.lax.dot_general(xn, wu, _NT, preferred_element_type=F32)
        lane = jax.lax.broadcasted_iota(jnp.int32, (8, 128), 1)
        hid = jnp.where(lane >= (p + 1) * 128 - F, jax.nn.silu(g) * u, 0.0)
        y_v[0] += jnp.dot(hid.astype(BF16), wd, preferred_element_type=F32)

    def o_proj(u):
        y_v[1] += sum(jnp.dot(head_row(o_v, _v_slot(u + 8 * i)), wo_v[u, i], preferred_element_type=F32)
                      for i in range(4))

    copy_x = pltpu.make_async_copy(x_h, x_v, s_x.at[0])
    copy_wr = pltpu.make_async_copy(wr_h, wr_v, s_x.at[1])
    for odd in range(2):
        lo_k(0, odd)
    copy_f(1, FT - 1).start()
    copy_x.start()
    copy_wr.start()
    _loop(4 * LEAD - 1, lambda e: [lo_k(e + 1, odd) for odd in range(2)])
    copy_f(2, FT - 1).start()
    l_v[...] = jnp.zeros(l_v.shape, F32)
    o_v[...] = jnp.zeros(o_v.shape, F32)
    y_v[...] = jnp.zeros(y_v.shape, F32)

    def stream(i):
        for i0, i1 in zip(cuts, cuts[1:]):
            h0, start_hi = [e for e in hi if e[0] <= i0][-1]
            l0, start_lo = [e for e in lo if e[0] <= i0][-1]

            @pl.when((i >= i0) & (i < i1))
            def _():
                def pairs(t):
                    for odd in range(2):
                        start_hi((i - h0) * 4 + t, odd)
                        start_lo((i - l0) * 4 + t, odd)
                _loop(4 if i1 < steps else jnp.where(i < steps - 1, 4, 2), pairs)

        n = i - LAG

        @pl.when(n == 0)
        def _():
            copy_x.wait()
            copy_wr.wait()
            x = x_v[0].astype(F32)
            mean = jnp.mean(x, axis=-1, keepdims=True)
            var = jnp.mean(jnp.square(x - mean), axis=-1, keepdims=True)
            xn_v[...] = jnp.broadcast_to(((x - mean) / jnp.sqrt(var + 1e-5)).astype(BF16).astype(F32), (8, D))

        @pl.when((n >= 15) & (n < 47) & (_mod(n - 15, 16) < 8))
        def _():
            j = _mod(_div(n - 15, 16) * 8 + _mod(n - 15, 8) + 12, 16)
            pl.when(_mod(j, 4) == 0)(lambda: wait_all(wq_v.at[_div(j, 4)], s_q.at[_div(j, 4)]))
            q_proj(j)

        pl.when(n == f0 + 31)(lambda: wait_all(wf_v, s_f.at[0]))
        pl.when((n >= f0 + 31) & (n < f0 + 31 + FP))(lambda: ffn(n - (f0 + 31)))

        @pl.when(n == f0 + 31 + FP)
        def _():
            xn = xn_v[...]
            r = jnp.sum(xn * wr_v[...].reshape(1, D).astype(F32), axis=-1, keepdims=True)
            y_v[0] = jax.nn.silu(xn + (xn * 0.0 + y_v[0] * jax.nn.sigmoid(r)))

        @pl.when(i >= steps - 4)
        def _():
            j = i - (steps - 4)
            c_v[j] = jnp.broadcast_to(head_row(o_v, _v_slot(8 * j)).astype(F32)[0:1], (DH, DH)).T

    tail = TAIL.split()
    e0, v0 = (steps - 1 - hi[-1][0]) * 4 + 2, NU - (LEAD + LAG - 3)
    first = [sum(int(t[0]) for t in tail[:j]) for j in range(len(tail) + 1)]
    chunks, quads = iter(range(8, 8 + NU - v0)), iter(QUADS)
    work = [next(chunks) if t[1] == "v" else next(quads) if t[1] == "o" else 0 for t in tail]
    assert e0 + first[-1] == 88 and e0 + first[work.index(2) + 1] >= 80 and not list(chunks) + list(quads)
    assert steps - LAG + VH == NU + v0 and LAG + Q0 + C1 + VH <= steps - 4

    def step(i):
        pl.when(i < steps)(lambda: stream(i))
        s = i - steps
        w = jnp.where(s >= 0, _pick(s, work), 0)

        @pl.when(s >= 0)
        def _():
            e = _pick(s, first)
            _loop(_pick(s + 1, first) - e, lambda t: [hi_wo(e0 + e + t, odd) for odd in range(2)])
            pl.when(w == 0)(lambda: pl.delay(T_IDLE))

        e = i - (LAG + Q0)
        done = jnp.where(s >= 0, NU + v0 + w - 8, e + jnp.clip(e - C0, 0, Q0 - 1) + jnp.clip(e - C1, 0, VH + 1))

        two = ((e >= C0) & (e < C0 + Q0 - 1)) | ((e >= C1) & (e < C1 + VH + 1))

        def chunk(j):
            for a in range(2):
                pl.when(_div(done + j, NU) == a)(lambda: attend(a, done + j - a * NU))

        _loop(jnp.where(s >= 0, _div(w, 8), jnp.where(e < 0, 0, jnp.where(two, 2, 1))), chunk)

        @pl.when((w > 0) & (w < 8))
        def _():
            wait_all(wo_v.at[w], s_o.at[w])
            o_proj(w)

    _loop(steps + len(tail), step)

    part = jnp.where(jax.lax.broadcasted_iota(jnp.int32, (8, D), 0) == 0, y_v[1], 0.0)
    gate = y_v[0]
    x = jnp.broadcast_to(x_v[0].astype(F32), (8, D))
    for i in VPU_ORDER:
        rows = _ds(i, 16)
        wait_all(wo_v.at[0, :, rows, :], s_o.at[8 + i])
        for j in range(4):
            prod = wo_v[0, j, rows, :].astype(F32) * jnp.concatenate([c_v[j, rows, :]] * (D // DH), axis=1)
            part = part + (prod[0:8] + prod[8:16])
    res = x + jnp.broadcast_to(jnp.sum(part, axis=0, keepdims=True), (8, D)) * gate
    out_ref[0] = res.astype(out_ref.dtype)[0:1]


@jax.jit
def pallas_recurrent_scan__sliding_block_cached__moe_arch_mod__decode_kernel(
    A_x: jax.Array,
    A_k_cache: jax.Array,
    A_v_cache: jax.Array,
    A_wq: jax.Array,
    A_wo: jax.Array,
    B_x: jax.Array,
    B_w_r: jax.Array,
    B_w_gate: jax.Array,
    B_w_up: jax.Array,
    B_w_down: jax.Array,
):
    del B_x
    hbm = pl.BlockSpec(memory_space=pltpu.HBM)
    dma = pltpu.SemaphoreType.DMA
    return pl.pallas_call(
        _kernel,
        out_shape=jax.ShapeDtypeStruct((1, 1, D), BF16),
        in_specs=[hbm] * 9,
        out_specs=pl.BlockSpec(memory_space=pltpu.VMEM),
        scratch_shapes=[
            pltpu.VMEM((1, 1, D), BF16),
            pltpu.VMEM((D,), BF16),
            pltpu.VMEM((4, 4, D // 4, 1024), BF16),
            pltpu.VMEM((2, NH, W + 16, DH), BF16),
            pltpu.VMEM((8, 4, DH, D), BF16),
            pltpu.VMEM((3, F, D), BF16),
            pltpu.VMEM((8, D), F32),
            pltpu.VMEM((NH, DH), F32),
            pltpu.VMEM((NC, CK // 128, NH, 128), F32),
            pltpu.VMEM((NH, 128), F32),
            pltpu.VMEM((NH, 128), F32),
            pltpu.VMEM((NH, DH), F32),
            pltpu.VMEM((2, 8, D), F32),
            pltpu.VMEM((4, DH, DH), F32),
            dma((2,)), dma((4,)), dma((2 * NU,)), dma((1,)), dma((16,)),
        ],
        compiler_params=pltpu.CompilerParams(
            vmem_limit_bytes=100 * 1024 * 1024,
            disable_bounds_checks=True,
            disable_semaphore_checks=True,
        ),
    )(A_x, A_k_cache, A_v_cache, A_wq.reshape(4, D // 4, NH * DH), A_wo.reshape(4, 8, DH, D), B_w_r,
      B_w_gate.T.reshape(2, F // 2, D), B_w_up.T.reshape(2, F // 2, D), B_w_down.reshape(2, F // 2, D))
```

```python
import jax
import jax.numpy as jnp
import jax.experimental.pallas as pl
import jax.experimental.pallas.tpu as pltpu

D = 512
NH = 32
DH = 128
SK = 32768
W = min(4096, max(256, SK // 4))
F = 1376

CK = 256
NC = W // CK
NU = 4 * NC
VH = 9
SHIFT = 1
FT = F // 16
FP = -(-F // 128)
LEAD = 3
LAG = 4
Q0 = 23
C0, C1 = 16, 52
TAIL = "0v 0v 0o 0o 0o 1v 0- 3v 2o 2- 2o 1o 3o"
QUADS = (5, 6, 7, 1, 3, 2, 4)
T_IDLE = 85
VPU_ORDER = (0, 1, 4, 2, 5, 3, 6, 7)

BF16 = jnp.bfloat16
F32 = jnp.float32
_NT = (((1,), (1,)), ((), ()))


def _div(n, d):
    return n // d if isinstance(n, int) else jax.lax.shift_right_logical(n, d.bit_length() - 1)


def _mod(n, d):
    return n & (d - 1)


def _ds(i, n):
    return pl.ds(i * n if isinstance(i, int) else pl.multiple_of(i * n, n), n)


def _k_head(slot):
    return (_div(slot, 8) * 4 + _mod(slot, 4)) ^ ((slot & 4) * 6)


def _v_head(slot):
    return _mod((((slot & 11) + _div(slot, 16) * 4) ^ ((slot & 4) * 6)) + SHIFT, NH)


def _v_slot(head):
    h = _mod(head + NH - SHIFT, NH)
    low = h ^ (_div(h, 16) * 24)
    return (low & 11) + (low & 4) * 4 + _div(h, 16) * 4


def _pick(s, table):
    word = [sum(v << 4 * j for j, v in enumerate(table[k:k + 8])) for k in (0, 8)]
    word = [w - (w >> 31 << 32) for w in word]
    return (jnp.where(s < 8, *word) >> 4 * _mod(s, 8)) & 15


def _loop(n, body):
    def body1(i, carry):
        body(i)
        return carry
    jax.lax.fori_loop(0, n, body1, 0)


def _kernel(x_h, k_h, v_h, wq_h, wo_h, wr_h, wg_h, wu_h, wd_h, out_ref,
            x_v, wr_v, wq_v, kv_v, wo_v, wf_v, xn_v, q_v, s_v, m_v, l_v, o_v, y_v, c_v,
            s_x, s_q, s_kv, s_f, s_o):
    def wait_all(buf, sem):
        pltpu.make_async_copy(buf, buf, sem).wait()

    def copy_kv(a, head, slot, n, r):
        return pltpu.make_async_copy((k_h, v_h)[a].at[0, pl.ds(head, n), _ds((SK - W) // 64 + r, 64), :],
                                     kv_v.at[a, pl.ds(slot, n), _ds(r, 64), :],
                                     s_kv.at[a * NU + _div(slot, 8) * NC + _div(r, 4)])

    def copy_wo(u, heads, rows, sem):
        return pltpu.make_async_copy(wo_h.at[heads, u, rows, :], wo_v.at[u, heads, rows, :], sem)

    def copy_f(a, r):
        return pltpu.make_async_copy((wg_h, wu_h, wd_h)[a].at[_mod(r, 2), _ds(_div(r, 2), 16), :],
                                     wf_v.at[a, _ds(r, 16), :], s_f.at[0])

    def lo_k(e, odd):
        slot = _div(e, 128) * 16 + _mod(e, 2) * 8 + 4 * odd
        copy_kv(0, _k_head(slot), slot, 4, _mod(_div(e, 2), 64)).start(priority=1)

    def lo_v2(e, odd):
        copy_kv(1, _v_head(16), 16, 4, e + odd * 4 * (NC - VH)).start(priority=1)

    def lo_v(e, odd):
        slot = _mod(_div(e, 64) + 3, 4) * 8 + 4 * odd
        copy_kv(1, _v_head(slot), slot, 4, _mod(e, 64)).start(priority=1)

    def lo_wo(e, odd):
        vpu = e >= 8
        u = jnp.where(vpu, 0, 3 + _div(e, 4))
        r = jnp.where(vpu, e - 6, _mod(e, 4)) * 2 + odd
        copy_wo(u, slice(None), _ds(r, 16), s_o.at[jnp.where(vpu, 8 + r, u)]).start(priority=1)

    def hi_wq(e, odd):
        j = _mod(_div(e, 64) * 2 + _mod(_div(e, 2), 2) + 3, 4)
        a, rows = _mod(e, 2) * 2 + odd, _ds(_mod(_div(e, 4), 16), 8)
        pltpu.make_async_copy(wq_h.at[a, rows, _ds(j, 1024)], wq_v.at[j, a, rows, :], s_q.at[j]).start()

    def hi_v(e, odd):
        slot = jnp.where(e < 128, 20, 16) + _mod(e, 2) * 2 + odd
        r = _div(e, 2) - jnp.where(e < 128, 0, 8 * VH - 64)
        copy_kv(1, _v_head(slot), slot, 1, r).start()

    def hi_f(e, odd):
        r = _div((2 * e + odd) * 171, 512)
        for a in range(3):
            pl.when(2 * e + odd - 3 * r == a)(lambda: copy_f(a, r).start())

    def hi_wo(e, odd):
        u, r = _pick(_div(e, 16), (5, 6, 7, 1, 2, 0)), _mod(e, 16)
        copy_wo(u, _ds(odd, 2), _ds(r, 8), s_o.at[jnp.where(u == 0, 8 + _div(r, 2), u)]).start()

    f0 = 32 + 4 * VH
    hi = [(0, hi_wq), (32, hi_v), (f0, hi_f), (f0 + 32, hi_wo)]
    lo = [(-LEAD, lo_k), (NU - LEAD, lo_v2), (NU + NC - VH - LEAD, lo_v), (2 * NU - VH - LEAD, lo_wo)]
    steps = lo[-1][0] + 3
    cuts = sorted({i for i, _ in hi + lo if i >= 0} | {steps})

    def head_row(ref, r):
        return jnp.broadcast_to(ref[pl.ds(r, 1), :], (8, DH)).astype(BF16)

    def q_proj(j):
        w = wq_v[_div(j, 4), :, :, _ds(_mod(j, 4), 256)].reshape(D, 256)
        q = jnp.dot(xn_v[...].astype(BF16), w, preferred_element_type=F32)
        for t in range(2):
            q_v[pl.ds(2 * j + t, 1), :] = q[0:1, t * DH:(t + 1) * DH]

    def qk(b, c):
        for i in range(8):
            h = _k_head(8 * b + i)
            s = jax.lax.dot_general(head_row(q_v, h), kv_v[0, 8 * b + i, _ds(c, CK), :], _NT,
                                    preferred_element_type=F32) * DH ** -0.5
            for j in range(CK // 128):
                s_v[c, j, pl.ds(_v_slot(h), 1), :] = s[0:1, j * 128:(j + 1) * 128]

    def pv(b, c):
        rows = _ds(b, 8)
        p = [jnp.exp(s_v[c, j, rows, :] - m_v[rows, :]) for j in range(CK // 128)]
        l_v[rows, :] += sum(p)
        p = jnp.concatenate(p, axis=1).astype(BF16)
        row = jax.lax.broadcasted_iota(jnp.int32, (8, DH), 0)
        o = None
        for i in range(8):
            t = jnp.dot(p, kv_v[1, 8 * b + i, _ds(c, CK), :], preferred_element_type=F32)
            o = t if o is None else jnp.where(row == i, t, o)
        o_v[rows, :] += o

        @pl.when(c == NC - 1)
        def _():
            o_v[rows, :] = o_v[rows, :] / jnp.sum(l_v[rows, :], axis=-1, keepdims=True)

    def attend(a, u):
        if a == 0:
            b, c = _div(u, 2 * NC) * 2 + _mod(u, 2), _mod(_div(u, 2), NC)
        else:
            b, c = _mod(_div(u, NC) + 2, 4), _mod(u, NC)
        wait_all(kv_v.at[a, _ds(b, 8), _ds(c, CK), :], s_kv.at[a * NU + b * NC + c])
        (qk, pv)[a](b, c)

        if a == 0:
            @pl.when(u == NU - 1)
            def _():
                m = jax.lax.fori_loop(0, NC, lambda c, m: jnp.maximum(m, jnp.max(s_v[c], axis=0)),
                                      jnp.full((NH, 128), -jnp.inf, F32))
                m_v[...] = jnp.broadcast_to(jnp.max(m, axis=-1, keepdims=True), (NH, 128))

    def ffn(p):
        wg, wu, wd = [wf_v[a, pl.ds(pl.multiple_of(jnp.minimum(128 * p, F - 128), 16), 128), :] for a in range(3)]
        xn = xn_v[...].astype(BF16)
        g = jax.lax.dot_general(xn, wg, _NT, preferred_element_type=F32)
        u = jax.lax.dot_general(xn, wu, _NT, preferred_element_type=F32)
        lane = jax.lax.broadcasted_iota(jnp.int32, (8, 128), 1)
        hid = jnp.where(lane >= (p + 1) * 128 - F, jax.nn.silu(g) * u, 0.0)
        y_v[0] += jnp.dot(hid.astype(BF16), wd, preferred_element_type=F32)

    def o_proj(u):
        y_v[1] += sum(jnp.dot(head_row(o_v, _v_slot(u + 8 * i)), wo_v[u, i], preferred_element_type=F32)
                      for i in range(4))

    copy_x = pltpu.make_async_copy(x_h, x_v, s_x.at[0])
    copy_wr = pltpu.make_async_copy(wr_h, wr_v, s_x.at[1])
    for odd in range(2):
        lo_k(0, odd)
    copy_f(1, FT - 1).start()
    copy_x.start()
    copy_wr.start()
    _loop(4 * LEAD - 1, lambda e: [lo_k(e + 1, odd) for odd in range(2)])
    copy_f(2, FT - 1).start()
    l_v[...] = jnp.zeros(l_v.shape, F32)
    o_v[...] = jnp.zeros(o_v.shape, F32)
    y_v[...] = jnp.zeros(y_v.shape, F32)

    def stream(i):
        for i0, i1 in zip(cuts, cuts[1:]):
            h0, start_hi = [e for e in hi if e[0] <= i0][-1]
            l0, start_lo = [e for e in lo if e[0] <= i0][-1]

            @pl.when((i >= i0) & (i < i1))
            def _():
                def pairs(t):
                    for odd in range(2):
                        start_hi((i - h0) * 4 + t, odd)
                        start_lo((i - l0) * 4 + t, odd)
                _loop(4 if i1 < steps else jnp.where(i < steps - 1, 4, 2), pairs)

        n = i - LAG

        @pl.when(n == 0)
        def _():
            copy_x.wait()
            copy_wr.wait()
            x = x_v[0].astype(F32)
            mean = jnp.mean(x, axis=-1, keepdims=True)
            var = jnp.mean(jnp.square(x - mean), axis=-1, keepdims=True)
            xn_v[...] = jnp.broadcast_to(((x - mean) / jnp.sqrt(var + 1e-5)).astype(BF16).astype(F32), (8, D))

        @pl.when((n >= 15) & (n < 47) & (_mod(n - 15, 16) < 8))
        def _():
            j = _mod(_div(n - 15, 16) * 8 + _mod(n - 15, 8) + 12, 16)
            pl.when(_mod(j, 4) == 0)(lambda: wait_all(wq_v.at[_div(j, 4)], s_q.at[_div(j, 4)]))
            q_proj(j)

        pl.when(n == f0 + 31)(lambda: wait_all(wf_v, s_f.at[0]))
        pl.when((n >= f0 + 31) & (n < f0 + 31 + FP))(lambda: ffn(n - (f0 + 31)))

        @pl.when(n == f0 + 31 + FP)
        def _():
            xn = xn_v[...]
            r = jnp.sum(xn * wr_v[...].reshape(1, D).astype(F32), axis=-1, keepdims=True)
            y_v[0] = jax.nn.silu(xn + (xn * 0.0 + y_v[0] * jax.nn.sigmoid(r)))

        @pl.when(i >= steps - 4)
        def _():
            j = i - (steps - 4)
            c_v[j] = jnp.broadcast_to(head_row(o_v, _v_slot(8 * j)).astype(F32)[0:1], (DH, DH)).T

    tail = TAIL.split()
    e0, v0 = (steps - 1 - hi[-1][0]) * 4 + 2, NU - (LEAD + LAG - 3)
    first = [sum(int(t[0]) for t in tail[:j]) for j in range(len(tail) + 1)]
    chunks, quads = iter(range(8, 8 + NU - v0)), iter(QUADS)
    work = [next(chunks) if t[1] == "v" else next(quads) if t[1] == "o" else 0 for t in tail]
    assert e0 + first[-1] == 88 and e0 + first[work.index(2) + 1] >= 80 and not list(chunks) + list(quads)
    assert steps - LAG + VH == NU + v0 and LAG + Q0 + C1 + VH < steps - 4

    def step(i):
        pl.when(i < steps)(lambda: stream(i))
        s = i - steps
        w = jnp.where(s >= 0, _pick(s, work), 0)

        @pl.when(s >= 0)
        def _():
            e = _pick(s, first)
            _loop(_pick(s + 1, first) - e, lambda t: [hi_wo(e0 + e + t, odd) for odd in range(2)])
            pl.when(w == 0)(lambda: pl.delay(T_IDLE))

        e = i - (LAG + Q0)
        done = jnp.where(s >= 0, NU + v0 + w - 8, e + jnp.clip(e - C0, 0, Q0 - 1) + jnp.clip(e - C1, 0, VH + 1))

        two = ((e >= C0) & (e < C0 + Q0 - 1)) | ((e >= C1) & (e < C1 + VH + 1))

        def chunk(j):
            for a in range(2):
                pl.when(_div(done + j, NU) == a)(lambda: attend(a, done + j - a * NU))

        _loop(jnp.where(s >= 0, _div(w, 8), jnp.where(e < 0, 0, jnp.where(two, 2, 1))), chunk)

        @pl.when((w > 0) & (w < 8))
        def _():
            wait_all(wo_v.at[w], s_o.at[w])
            o_proj(w)

    _loop(steps + len(tail), step)

    part = jnp.where(jax.lax.broadcasted_iota(jnp.int32, (8, D), 0) == 0, y_v[1], 0.0)
    gate = y_v[0]
    x = jnp.broadcast_to(x_v[0].astype(F32), (8, D))
    for i in VPU_ORDER:
        rows = _ds(i, 16)
        wait_all(wo_v.at[0, :, rows, :], s_o.at[8 + i])
        for j in range(4):
            prod = wo_v[0, j, rows, :].astype(F32) * jnp.concatenate([c_v[j, rows, :]] * (D // DH), axis=1)
            part = part + (prod[0:8] + prod[8:16])
    res = x + jnp.broadcast_to(jnp.sum(part, axis=0, keepdims=True), (8, D)) * gate
    out_ref[0] = res.astype(out_ref.dtype)[0:1]


@jax.jit
def pallas_recurrent_scan__sliding_block_cached__moe_arch_mod__decode_kernel(
    A_x: jax.Array,
    A_k_cache: jax.Array,
    A_v_cache: jax.Array,
    A_wq: jax.Array,
    A_wo: jax.Array,
    B_x: jax.Array,
    B_w_r: jax.Array,
    B_w_gate: jax.Array,
    B_w_up: jax.Array,
    B_w_down: jax.Array,
):
    del B_x
    hbm = pl.BlockSpec(memory_space=pltpu.HBM)
    dma = pltpu.SemaphoreType.DMA
    return pl.pallas_call(
        _kernel,
        out_shape=jax.ShapeDtypeStruct((1, 1, D), BF16),
        in_specs=[hbm] * 9,
        out_specs=pl.BlockSpec(memory_space=pltpu.VMEM),
        scratch_shapes=[
            pltpu.VMEM((1, 1, D), BF16),
            pltpu.VMEM((D,), BF16),
            pltpu.VMEM((4, 4, D // 4, 1024), BF16),
            pltpu.VMEM((2, NH, W + 16, DH), BF16),
            pltpu.VMEM((8, 4, DH, D), BF16),
            pltpu.VMEM((3, F, D), BF16),
            pltpu.VMEM((8, D), F32),
            pltpu.VMEM((NH, DH), F32),
            pltpu.VMEM((NC, CK // 128, NH, 128), F32),
            pltpu.VMEM((NH, 128), F32),
            pltpu.VMEM((NH, 128), F32),
            pltpu.VMEM((NH, DH), F32),
            pltpu.VMEM((2, 8, D), F32),
            pltpu.VMEM((4, DH, DH), F32),
            dma((2,)), dma((4,)), dma((2 * NU,)), dma((1,)), dma((16,)),
        ],
        compiler_params=pltpu.CompilerParams(
            vmem_limit_bytes=100 * 1024 * 1024,
            disable_bounds_checks=True,
            disable_semaphore_checks=True,
        ),
    )(A_x, A_k_cache, A_v_cache, A_wq.reshape(4, D // 4, NH * DH), A_wo.reshape(4, 8, DH, D), B_w_r,
      B_w_gate.T.reshape(2, F // 2, D), B_w_up.T.reshape(2, F // 2, D), B_w_down.reshape(2, F // 2, D))
```

```python
import jax
import jax.numpy as jnp
import jax.experimental.pallas as pl
import jax.experimental.pallas.tpu as pltpu

D = 512
NH = 32
DH = 128
SK = 32768
W = min(4096, max(256, SK // 4))
F = 1376

CK = 256
NC = W // CK
NU = 4 * NC
VH = 9
SHIFT = 1
FT = F // 16
FP = -(-F // 128)
LEAD = 3
LAG = 4
Q0 = 23
C0, C1 = 16, 52
TAIL = "0v 0v 0o 0o 0o 1v 0- 3v 2o 2- 2o 1o 3o"
QUADS = (5, 6, 7, 1, 3, 2, 4)
T_IDLE = 85
VPU_ORDER = (0, 1, 4, 2, 5, 3, 6, 7)

BF16 = jnp.bfloat16
F32 = jnp.float32
_NT = (((1,), (1,)), ((), ()))


def _div(n, d):
    return n // d if isinstance(n, int) else jax.lax.shift_right_logical(n, d.bit_length() - 1)


def _mod(n, d):
    return n & (d - 1)


def _ds(i, n):
    return pl.ds(i * n if isinstance(i, int) else pl.multiple_of(i * n, n), n)


def _k_head(slot):
    return (_div(slot, 8) * 4 + _mod(slot, 4)) ^ ((slot & 4) * 6)


def _v_head(slot):
    return _mod((((slot & 11) + _div(slot, 16) * 4) ^ ((slot & 4) * 6)) + SHIFT, NH)


def _v_slot(head):
    h = _mod(head + NH - SHIFT, NH)
    low = h ^ (_div(h, 16) * 24)
    return (low & 11) + (low & 4) * 4 + _div(h, 16) * 4


def _pick(s, table):
    word = [sum(v << 4 * j for j, v in enumerate(table[k:k + 8])) for k in (0, 8)]
    word = [w - (w >> 31 << 32) for w in word]
    return (jnp.where(s < 8, *word) >> 4 * _mod(s, 8)) & 15


def _loop(n, body):
    def body1(i, carry):
        body(i)
        return carry
    jax.lax.fori_loop(0, n, body1, 0)


def _kernel(x_h, k_h, v_h, wq_h, wo_h, wr_h, wg_h, wu_h, wd_h, out_ref,
            x_v, wr_v, wq_v, kv_v, wo_v, wf_v, xn_v, q_v, s_v, m_v, l_v, o_v, y_v, c_v,
            s_x, s_q, s_kv, s_f, s_o):
    def wait_all(buf, sem):
        pltpu.make_async_copy(buf, buf, sem).wait()

    def copy_kv(a, head, slot, n, r):
        return pltpu.make_async_copy((k_h, v_h)[a].at[0, pl.ds(head, n), _ds((SK - W) // 64 + r, 64), :],
                                     kv_v.at[a, pl.ds(slot, n), _ds(r, 64), :],
                                     s_kv.at[a * NU + _div(slot, 8) * NC + _div(r, 4)])

    def copy_wo(u, heads, r):
        return pltpu.make_async_copy(wo_h.at[heads, u, _ds(r, 16), :], wo_v.at[u, heads, _ds(r, 16), :],
                                     s_o.at[jnp.where(u == 0, 8 + r, u)])

    def copy_f(a, r):
        return pltpu.make_async_copy((wg_h, wu_h, wd_h)[a].at[_mod(r, 2), _ds(_div(r, 2), 16), :],
                                     wf_v.at[a, _ds(r, 16), :], s_f.at[0])

    def lo_k(e, odd):
        slot = _div(e, 128) * 16 + _mod(e, 2) * 8 + 4 * odd
        copy_kv(0, _k_head(slot), slot, 4, _mod(_div(e, 2), 64)).start(priority=1)

    def lo_v2(e, odd):
        copy_kv(1, _v_head(16), 16, 4, e + odd * 4 * (NC - VH)).start(priority=1)

    def lo_v(e, odd):
        slot = _mod(_div(e, 64) + 3, 4) * 8 + 4 * odd
        copy_kv(1, _v_head(slot), slot, 4, _mod(e, 64)).start(priority=1)

    def lo_wo(e, odd):
        u, r = jnp.where(e < 8, 3 + _div(e, 4), 0), jnp.where(e < 8, _mod(e, 4), e - 6) * 2 + odd
        copy_wo(u, slice(None), r).start(priority=1)

    def hi_wq(e, odd):
        j = _mod(_div(e, 64) * 2 + _mod(_div(e, 2), 2) + 3, 4)
        a, rows = _mod(e, 2) * 2 + odd, _ds(_mod(_div(e, 4) + jnp.where(j == 0, 1, 0), 16), 8)
        pltpu.make_async_copy(wq_h.at[a, rows, _ds(j, 1024)], wq_v.at[j, a, rows, :], s_q.at[j]).start()

    def hi_v(e, odd):
        slot = jnp.where(e < 128, 20, 16) + _mod(e, 2) * 2 + odd
        r = _div(e, 2) - jnp.where(e < 128, 0, 8 * VH - 64)
        copy_kv(1, _v_head(slot), slot, 1, r).start()

    def hi_f(e, odd):
        r = _div((2 * e + odd) * 171, 512)
        for a in range(3):
            pl.when(2 * e + odd - 3 * r == a)(lambda: copy_f(a, r).start())

    def hi_wo(e, odd):
        u = _pick(jnp.where(e < 64, _div(e, 32) * 2 + _mod(_div(e, 2), 2), _div(e, 16)), (5, 1, 6, 7, 2, 0))
        r = _mod(jnp.where(e < 64, _div(e, 4), _div(e, 2)), 8)
        copy_wo(u, _mod(e, 2) * 2 + odd, r).start()

    f0 = 32 + 4 * VH
    hi = [(0, hi_wq), (32, hi_v), (f0, hi_f), (f0 + 32, hi_wo)]
    lo = [(-LEAD, lo_k), (NU - LEAD, lo_v2), (NU + NC - VH - LEAD, lo_v), (2 * NU - VH - LEAD, lo_wo)]
    steps = lo[-1][0] + 3
    cuts = sorted({i for i, _ in hi + lo if i >= 0} | {steps})

    def head_row(ref, r):
        return jnp.broadcast_to(ref[pl.ds(r, 1), :], (8, DH)).astype(BF16)

    def q_proj(j):
        w = wq_v[_div(j, 4), :, :, _ds(_mod(j, 4), 256)].reshape(D, 256)
        q = jnp.dot(xn_v[...].astype(BF16), w, preferred_element_type=F32)
        for t in range(2):
            q_v[pl.ds(2 * j + t, 1), :] = q[0:1, t * DH:(t + 1) * DH]

    def qk(b, c):
        for i in range(8):
            h = _k_head(8 * b + i)
            s = jax.lax.dot_general(head_row(q_v, h), kv_v[0, 8 * b + i, _ds(c, CK), :], _NT,
                                    preferred_element_type=F32) * DH ** -0.5
            for j in range(CK // 128):
                s_v[c, j, pl.ds(_v_slot(h), 1), :] = s[0:1, j * 128:(j + 1) * 128]

    def pv(b, c):
        rows = _ds(b, 8)
        p = [jnp.exp(s_v[c, j, rows, :] - m_v[rows, :]) for j in range(CK // 128)]
        l_v[rows, :] += sum(p)
        p = jnp.concatenate(p, axis=1).astype(BF16)
        row = jax.lax.broadcasted_iota(jnp.int32, (8, DH), 0)
        o = None
        for i in range(8):
            t = jnp.dot(p, kv_v[1, 8 * b + i, _ds(c, CK), :], preferred_element_type=F32)
            o = t if o is None else jnp.where(row == i, t, o)
        o_v[rows, :] += o

        @pl.when(c == NC - 1)
        def _():
            o_v[rows, :] = o_v[rows, :] / jnp.sum(l_v[rows, :], axis=-1, keepdims=True)

    def attend(a, u):
        if a == 0:
            b, c = _div(u, 2 * NC) * 2 + _mod(u, 2), _mod(_div(u, 2), NC)
        else:
            b, c = _mod(_div(u, NC) + 2, 4), _mod(u, NC)
        wait_all(kv_v.at[a, _ds(b, 8), _ds(c, CK), :], s_kv.at[a * NU + b * NC + c])
        (qk, pv)[a](b, c)

        if a == 0:
            @pl.when(u == NU - 1)
            def _():
                m = jax.lax.fori_loop(0, NC, lambda c, m: jnp.maximum(m, jnp.max(s_v[c], axis=0)),
                                      jnp.full((NH, 128), -jnp.inf, F32))
                m_v[...] = jnp.broadcast_to(jnp.max(m, axis=-1, keepdims=True), (NH, 128))

    def ffn(p):
        wg, wu, wd = [wf_v[a, pl.ds(pl.multiple_of(jnp.minimum(128 * p, F - 128), 16), 128), :] for a in range(3)]
        xn = xn_v[...].astype(BF16)
        g = jax.lax.dot_general(xn, wg, _NT, preferred_element_type=F32)
        u = jax.lax.dot_general(xn, wu, _NT, preferred_element_type=F32)
        lane = jax.lax.broadcasted_iota(jnp.int32, (8, 128), 1)
        hid = jnp.where(lane >= (p + 1) * 128 - F, jax.nn.silu(g) * u, 0.0)
        y_v[0] += jnp.dot(hid.astype(BF16), wd, preferred_element_type=F32)

    def o_proj(u):
        y_v[1] += sum(jnp.dot(head_row(o_v, _v_slot(u + 8 * i)), wo_v[u, i], preferred_element_type=F32)
                      for i in range(4))

    copy_x = pltpu.make_async_copy(x_h, x_v, s_x.at[0])
    copy_wr = pltpu.make_async_copy(wr_h, wr_v, s_x.at[1])
    for odd in range(2):
        lo_k(0, odd)
    copy_f(1, FT - 1).start()

    def lead(e):
        for odd in range(2):
            lo_k(e + 1, odd)
        pl.when(e == 7)(lambda: copy_f(2, FT - 1).start())

    _loop(4 * LEAD - 1, lead)
    copy_x.start()
    copy_wr.start()
    l_v[...] = jnp.zeros(l_v.shape, F32)
    o_v[...] = jnp.zeros(o_v.shape, F32)
    y_v[...] = jnp.zeros(y_v.shape, F32)

    def stream(i):
        for i0, i1 in zip(cuts, cuts[1:]):
            h0, start_hi = [e for e in hi if e[0] <= i0][-1]
            l0, start_lo = [e for e in lo if e[0] <= i0][-1]

            @pl.when((i >= i0) & (i < i1))
            def _():
                def pairs(t):
                    for odd in range(2):
                        start_hi((i - h0) * 4 + t, odd)
                        start_lo((i - l0) * 4 + t, odd)
                _loop(4 if i1 < steps else jnp.where(i < steps - 1, 4, 2), pairs)

        n = i - LAG

        @pl.when(n == 0)
        def _():
            copy_x.wait()
            copy_wr.wait()
            x = x_v[0].astype(F32)
            mean = jnp.mean(x, axis=-1, keepdims=True)
            var = jnp.mean(jnp.square(x - mean), axis=-1, keepdims=True)
            xn_v[...] = jnp.broadcast_to(((x - mean) / jnp.sqrt(var + 1e-5)).astype(BF16).astype(F32), (8, D))

        @pl.when((n >= 15) & (n < 47) & (_mod(n - 15, 16) < 8))
        def _():
            j = _mod(_div(n - 15, 16) * 8 + _mod(n - 15, 8) + 12, 16)
            pl.when(_mod(j, 4) == 0)(lambda: wait_all(wq_v.at[_div(j, 4)], s_q.at[_div(j, 4)]))
            q_proj(j)

        pl.when(n == f0 + 31)(lambda: wait_all(wf_v, s_f.at[0]))
        pl.when((n >= f0 + 31) & (n < f0 + 31 + FP))(lambda: ffn(n - (f0 + 31)))

        @pl.when(n == f0 + 31 + FP)
        def _():
            xn = xn_v[...]
            r = jnp.sum(xn * wr_v[...].reshape(1, D).astype(F32), axis=-1, keepdims=True)
            y_v[0] = jax.nn.silu(xn + (xn * 0.0 + y_v[0] * jax.nn.sigmoid(r)))

        @pl.when(i >= steps - 4)
        def _():
            j = i - (steps - 4)
            c_v[j] = jnp.broadcast_to(head_row(o_v, _v_slot(8 * j)).astype(F32)[0:1], (DH, DH)).T

    tail = TAIL.split()
    e0, v0 = (steps - 1 - hi[-1][0]) * 4 + 2, NU - (LEAD + LAG - 3)
    first = [sum(int(t[0]) for t in tail[:j]) for j in range(len(tail) + 1)]
    chunks, quads = iter(range(8, 8 + NU - v0)), iter(QUADS)
    work = [next(chunks) if t[1] == "v" else next(quads) if t[1] == "o" else 0 for t in tail]
    assert e0 + first[-1] == 88 and e0 + first[work.index(2) + 1] >= 80 and not list(chunks) + list(quads)
    assert steps - LAG + VH == NU + v0 and LAG + Q0 + C1 + VH < steps - 4

    def step(i):
        pl.when(i < steps)(lambda: stream(i))
        s = i - steps
        w = jnp.where(s >= 0, _pick(s, work), 0)

        @pl.when(s >= 0)
        def _():
            e = _pick(s, first)
            _loop(_pick(s + 1, first) - e, lambda t: [hi_wo(e0 + e + t, odd) for odd in range(2)])
            pl.when(w == 0)(lambda: pl.delay(T_IDLE))

        e = i - (LAG + Q0)
        done = jnp.where(s >= 0, NU + v0 + w - 8, e + jnp.clip(e - C0, 0, Q0 - 1) + jnp.clip(e - C1, 0, VH + 1))

        two = ((e >= C0) & (e < C0 + Q0 - 1)) | ((e >= C1) & (e < C1 + VH + 1))

        def chunk(j):
            for a in range(2):
                pl.when(_div(done + j, NU) == a)(lambda: attend(a, done + j - a * NU))

        _loop(jnp.where(s >= 0, _div(w, 8), jnp.where(e < 0, 0, jnp.where(two, 2, 1))), chunk)

        @pl.when((w > 0) & (w < 8))
        def _():
            wait_all(wo_v.at[w], s_o.at[w])
            o_proj(w)

    _loop(steps + len(tail), step)

    part = jnp.where(jax.lax.broadcasted_iota(jnp.int32, (8, D), 0) == 0, y_v[1], 0.0)
    gate = y_v[0]
    x = jnp.broadcast_to(x_v[0].astype(F32), (8, D))
    for i in VPU_ORDER:
        rows = _ds(i, 16)
        wait_all(wo_v.at[0, :, rows, :], s_o.at[8 + i])
        for j in range(4):
            prod = wo_v[0, j, rows, :].astype(F32) * jnp.concatenate([c_v[j, rows, :]] * (D // DH), axis=1)
            part = part + (prod[0:8] + prod[8:16])
    res = x + jnp.broadcast_to(jnp.sum(part, axis=0, keepdims=True), (8, D)) * gate
    out_ref[0] = res.astype(out_ref.dtype)[0:1]


@jax.jit
def pallas_recurrent_scan__sliding_block_cached__moe_arch_mod__decode_kernel(
    A_x: jax.Array,
    A_k_cache: jax.Array,
    A_v_cache: jax.Array,
    A_wq: jax.Array,
    A_wo: jax.Array,
    B_x: jax.Array,
    B_w_r: jax.Array,
    B_w_gate: jax.Array,
    B_w_up: jax.Array,
    B_w_down: jax.Array,
):
    del B_x
    hbm = pl.BlockSpec(memory_space=pltpu.HBM)
    dma = pltpu.SemaphoreType.DMA
    return pl.pallas_call(
        _kernel,
        out_shape=jax.ShapeDtypeStruct((1, 1, D), BF16),
        in_specs=[hbm] * 9,
        out_specs=pl.BlockSpec(memory_space=pltpu.VMEM),
        scratch_shapes=[
            pltpu.VMEM((1, 1, D), BF16),
            pltpu.VMEM((D,), BF16),
            pltpu.VMEM((4, 4, D // 4, 1024), BF16),
            pltpu.VMEM((2, NH, W, DH), BF16),
            pltpu.VMEM((8, 4, DH, D), BF16),
            pltpu.VMEM((3, F, D), BF16),
            pltpu.VMEM((8, D), F32),
            pltpu.VMEM((NH, DH), F32),
            pltpu.VMEM((NC, CK // 128, NH, 128), F32),
            pltpu.VMEM((NH, 128), F32),
            pltpu.VMEM((NH, 128), F32),
            pltpu.VMEM((NH, DH), F32),
            pltpu.VMEM((2, 8, D), F32),
            pltpu.VMEM((4, DH, DH), F32),
            dma((2,)), dma((4,)), dma((2 * NU,)), dma((1,)), dma((16,)),
        ],
        compiler_params=pltpu.CompilerParams(
            vmem_limit_bytes=100 * 1024 * 1024,
            disable_bounds_checks=True,
            disable_semaphore_checks=True,
        ),
    )(A_x, A_k_cache, A_v_cache, A_wq.reshape(4, D // 4, NH * DH), A_wo.reshape(4, 8, DH, D), B_w_r,
      B_w_gate.T.reshape(2, F // 2, D), B_w_up.T.reshape(2, F // 2, D), B_w_down.reshape(2, F // 2, D))
```

```python
import jax
import jax.numpy as jnp
import jax.experimental.pallas as pl
import jax.experimental.pallas.tpu as pltpu

D = 512
NH = 32
DH = 128
SK = 32768
W = min(4096, max(256, SK // 4))
F = 1376

CK = 256
NC = W // CK
NU = 4 * NC
VH = 9
SHIFT = 1
FT = F // 16
FP = -(-F // 128)
LEAD = 3
LAG = 4
Q0 = 23
C0 = 10
TAIL = "0v 0v 0o 0o 0o 1v 0- 3v 2o 4o 1o 3o"
QUADS = (5, 6, 7, 1, 3, 2, 4)
T_IDLE = 85
VPU_ORDER = (0, 1, 4, 2, 5, 3, 6, 7)

BF16 = jnp.bfloat16
F32 = jnp.float32
_NT = (((1,), (1,)), ((), ()))


def _div(n, d):
    return n // d if isinstance(n, int) else jax.lax.shift_right_logical(n, d.bit_length() - 1)


def _mod(n, d):
    return n & (d - 1)


def _ds(i, n):
    return pl.ds(i * n if isinstance(i, int) else pl.multiple_of(i * n, n), n)


def _k_head(slot):
    return (_div(slot, 8) * 4 + _mod(slot, 4)) ^ ((slot & 4) * 6)


def _v_head(slot):
    return _mod((((slot & 11) + _div(slot, 16) * 4) ^ ((slot & 4) * 6)) + SHIFT, NH)


def _v_slot(head):
    h = _mod(head + NH - SHIFT, NH)
    low = h ^ (_div(h, 16) * 24)
    return (low & 11) + (low & 4) * 4 + _div(h, 16) * 4


def _pick(s, table):
    word = [sum(v << 4 * j for j, v in enumerate(table[k:k + 8])) for k in (0, 8)]
    word = [w - (w >> 31 << 32) for w in word]
    return (jnp.where(s < 8, *word) >> 4 * _mod(s, 8)) & 15


def _loop(n, body):
    def body1(i, carry):
        body(i)
        return carry
    jax.lax.fori_loop(0, n, body1, 0)


def _kernel(x_h, k_h, v_h, wq_h, wo_h, wr_h, wg_h, wu_h, wd_h, out_ref,
            x_v, wr_v, wq_v, kv_v, wo_v, wf_v, xn_v, q_v, s_v, m_v, l_v, o_v, y_v, c_v,
            s_x, s_q, s_kv, s_f, s_o):
    def wait_all(buf, sem):
        pltpu.make_async_copy(buf, buf, sem).wait()

    def copy_kv(a, head, slot, n, r):
        return pltpu.make_async_copy((k_h, v_h)[a].at[0, pl.ds(head, n), _ds((SK - W) // 64 + r, 64), :],
                                     kv_v.at[a, pl.ds(slot, n), _ds(r, 64), :],
                                     s_kv.at[a * NU + _div(slot, 8) * NC + _div(r, 4)])

    def copy_wo(u, heads, r):
        return pltpu.make_async_copy(wo_h.at[heads, u, _ds(r, 16), :], wo_v.at[u, heads, _ds(r, 16), :],
                                     s_o.at[jnp.where(u == 0, 8 + r, u)])

    def copy_f(a, r):
        return pltpu.make_async_copy((wg_h, wu_h, wd_h)[a].at[_mod(r, 2), _ds(_div(r, 2), 16), :],
                                     wf_v.at[a, _ds(r, 16), :], s_f.at[0])

    def lo_k(e, odd):
        slot = _div(e, 128) * 16 + _mod(e, 2) * 8 + 4 * odd
        copy_kv(0, _k_head(slot), slot, 4, _mod(_div(e, 2), 64)).start(priority=1)

    def lo_v2(e, odd):
        copy_kv(1, _v_head(16), 16, 4, e + odd * 4 * (NC - VH)).start(priority=1)

    def lo_v(e, odd):
        for j in range(2):
            slot = _mod(_div(e, 64) + 3, 4) * 8 + (0, 6, 4, 2)[2 * odd + j]
            copy_kv(1, _v_head(slot), slot, 2, _mod(e, 64)).start(priority=1)

    def lo_wo(e, odd):
        u, r = jnp.where(e < 8, 3 + _div(e, 4), 0), jnp.where(e < 8, _mod(e, 4), e - 6) * 2 + odd
        copy_wo(u, slice(None), r).start(priority=1)

    def hi_wq(e, odd):
        j = _mod(_div(e, 64) * 2 + _mod(_div(e, 2), 2) + 3, 4)
        a, rows = _mod(e, 2) * 2 + odd, _ds(_mod(_div(e, 4) + jnp.where(j == 0, 1, 0), 16), 8)
        pltpu.make_async_copy(wq_h.at[a, rows, _ds(j, 1024)], wq_v.at[j, a, rows, :], s_q.at[j]).start()

    def hi_v(e, odd):
        slot = jnp.where(e < 128, 20, 16) + _mod(e, 2) * 2 + odd
        r = _div(e, 2) - jnp.where(e < 128, 0, 8 * VH - 64)
        copy_kv(1, _v_head(slot), slot, 1, r).start()

    def hi_f(e, odd):
        r = _div((2 * e + odd) * 171, 512)
        for a in range(3):
            pl.when(2 * e + odd - 3 * r == a)(lambda: copy_f(a, r).start())

    def hi_wo(e, odd):
        u = _pick(jnp.where(e < 64, _div(e, 32) * 2 + _mod(_div(e, 2), 2), _div(e, 16)), (5, 1, 6, 7, 2, 0))
        r = _mod(jnp.where(e < 64, _div(e, 4), _div(e, 2)), 8)
        copy_wo(u, _mod(e, 2) * 2 + odd, r).start()

    f0 = 32 + 4 * VH
    hi = [(0, hi_wq), (32, hi_v), (f0, hi_f), (f0 + 32, hi_wo)]
    lo = [(i - LEAD, f) for i, f in ((0, lo_k), (NU, lo_v2), (NU + NC - VH, lo_v), (2 * NU - VH, lo_wo))]
    steps = lo[-1][0] + 3
    cuts = sorted({i for i, _ in hi + lo if i >= 0} | {steps})

    def head_row(ref, r):
        return jnp.broadcast_to(ref[pl.ds(r, 1), :], (8, DH)).astype(BF16)

    def q_proj(j):
        w = wq_v[_div(j, 4), :, :, _ds(_mod(j, 4), 256)].reshape(D, 256)
        q = jnp.dot(xn_v[...].astype(BF16), w, preferred_element_type=F32)
        for t in range(2):
            q_v[pl.ds(2 * j + t, 1), :] = q[0:1, t * DH:(t + 1) * DH]

    def qk(b, c):
        for i in range(8):
            h = _k_head(8 * b + i)
            s = jax.lax.dot_general(head_row(q_v, h), kv_v[0, 8 * b + i, _ds(c, CK), :], _NT,
                                    preferred_element_type=F32) * DH ** -0.5
            for j in range(CK // 128):
                s_v[c, j, pl.ds(_v_slot(h), 1), :] = s[0:1, j * 128:(j + 1) * 128]

    def pv(b, c):
        rows = _ds(b, 8)
        p = [jnp.exp(s_v[c, j, rows, :] - m_v[rows, :]) for j in range(CK // 128)]
        l_v[rows, :] += sum(p)
        p = jnp.concatenate(p, axis=1).astype(BF16)
        row = jax.lax.broadcasted_iota(jnp.int32, (8, DH), 0)
        o = None
        for i in range(8):
            t = jnp.dot(p, kv_v[1, 8 * b + i, _ds(c, CK), :], preferred_element_type=F32)
            o = t if o is None else jnp.where(row == i, t, o)
        o_v[rows, :] += o

        @pl.when(c == NC - 1)
        def _():
            o_v[rows, :] = o_v[rows, :] / jnp.sum(l_v[rows, :], axis=-1, keepdims=True)

    def attend(a, u):
        if a == 0:
            b, c = _div(u, 2 * NC) * 2 + _mod(u, 2), _mod(_div(u, 2), NC)
        else:
            b, c = _mod(_div(u, NC) + 2, 4), _mod(u, NC)
        wait_all(kv_v.at[a, _ds(b, 8), _ds(c, CK), :], s_kv.at[a * NU + b * NC + c])
        (qk, pv)[a](b, c)

        if a == 0:
            @pl.when(u == NU - 1)
            def _():
                m = jax.lax.fori_loop(0, NC, lambda c, m: jnp.maximum(m, jnp.max(s_v[c], axis=0)),
                                      jnp.full((NH, 128), -jnp.inf, F32))
                m_v[...] = jnp.broadcast_to(jnp.max(m, axis=-1, keepdims=True), (NH, 128))

    def ffn(p):
        wg, wu, wd = [wf_v[a, pl.ds(pl.multiple_of(jnp.minimum(128 * p, F - 128), 16), 128), :] for a in range(3)]
        xn = xn_v[...].astype(BF16)
        g = jax.lax.dot_general(xn, wg, _NT, preferred_element_type=F32)
        u = jax.lax.dot_general(xn, wu, _NT, preferred_element_type=F32)
        lane = jax.lax.broadcasted_iota(jnp.int32, (8, 128), 1)
        hid = jnp.where(lane >= (p + 1) * 128 - F, jax.nn.silu(g) * u, 0.0)
        y_v[0] += jnp.dot(hid.astype(BF16), wd, preferred_element_type=F32)

    def o_proj(u):
        y_v[1] += sum(jnp.dot(head_row(o_v, _v_slot(u + 8 * i)), wo_v[u, i], preferred_element_type=F32)
                      for i in range(4))

    copy_x = pltpu.make_async_copy(x_h, x_v, s_x.at[0])
    copy_wr = pltpu.make_async_copy(wr_h, wr_v, s_x.at[1])
    for odd in range(2):
        lo_k(0, odd)
    copy_f(1, FT - 1).start()

    def lead(e):
        for odd in range(2):
            lo_k(e + 1, odd)
        pl.when(e == 7)(lambda: copy_f(2, FT - 1).start())

    _loop(4 * LEAD - 1, lead)
    copy_x.start()
    copy_wr.start()
    l_v[...] = jnp.zeros(l_v.shape, F32)
    o_v[...] = jnp.zeros(o_v.shape, F32)
    y_v[...] = jnp.zeros(y_v.shape, F32)

    def stream(i):
        for i0, i1 in zip(cuts, cuts[1:]):
            h0, start_hi = [e for e in hi if e[0] <= i0][-1]
            l0, start_lo = [e for e in lo if e[0] <= i0][-1]

            @pl.when((i >= i0) & (i < i1))
            def _():
                def pairs(t):
                    for odd in range(2):
                        start_hi((i - h0) * 4 + t, odd)
                        start_lo((i - l0) * 4 + t, odd)
                _loop(4 if i1 < steps else jnp.where(i < steps - 1, 4, 2), pairs)

        n = i - LAG

        @pl.when(n == 0)
        def _():
            copy_x.wait()
            copy_wr.wait()
            x = x_v[0].astype(F32)
            mean = jnp.mean(x, axis=-1, keepdims=True)
            var = jnp.mean(jnp.square(x - mean), axis=-1, keepdims=True)
            xn_v[...] = jnp.broadcast_to(((x - mean) / jnp.sqrt(var + 1e-5)).astype(BF16).astype(F32), (8, D))

        @pl.when((n >= 15) & (n < 47) & (_mod(n - 15, 16) < 8))
        def _():
            j = _mod(_div(n - 15, 16) * 8 + _mod(n - 15, 8) + 12, 16)
            pl.when(_mod(j, 4) == 0)(lambda: wait_all(wq_v.at[_div(j, 4)], s_q.at[_div(j, 4)]))
            q_proj(j)

        pl.when(n == f0 + 31)(lambda: wait_all(wf_v, s_f.at[0]))
        pl.when((n >= f0 + 31) & (n < f0 + 31 + FP))(lambda: ffn(n - (f0 + 31)))

        @pl.when(n == f0 + 31 + FP)
        def _():
            xn = xn_v[...]
            r = jnp.sum(xn * wr_v[...].reshape(1, D).astype(F32), axis=-1, keepdims=True)
            y_v[0] = jax.nn.silu(xn + (xn * 0.0 + y_v[0] * jax.nn.sigmoid(r)))

        @pl.when(i >= steps - 4)
        def _():
            j = i - (steps - 4)
            c_v[j] = jnp.broadcast_to(head_row(o_v, _v_slot(8 * j)).astype(F32)[0:1], (DH, DH)).T

    tail = TAIL.split()
    e0, v0 = (steps - 1 - hi[-1][0]) * 4 + 2, NU - (LEAD + LAG - 3)
    first = [sum(int(t[0]) for t in tail[:j]) for j in range(len(tail) + 1)]
    chunks, quads = iter(range(8, 8 + NU - v0)), iter(QUADS)
    work = [next(chunks) if t[1] == "v" else next(quads) if t[1] == "o" else 0 for t in tail]
    assert e0 + first[-1] == 88 and e0 + first[work.index(2) + 1] >= 80 and not list(chunks) + list(quads)
    assert steps - LAG + VH == NU + v0 and LAG + C0 + 3 * Q0 + 2 * VH <= steps - 4

    def step(i):
        pl.when(i < steps)(lambda: stream(i))
        s = i - steps
        w = jnp.where(s >= 0, _pick(s, work), 0)

        @pl.when(s >= 0)
        def _():
            e = _pick(s, first)
            _loop(_pick(s + 1, first) - e, lambda t: [hi_wo(e0 + e + t, odd) for odd in range(2)])
            pl.when(w == 0)(lambda: pl.delay(T_IDLE))

        e = i - (LAG + Q0)
        done = jnp.where(s >= 0, NU + v0 + w - 8, e + jnp.clip(_div(e - C0 + 256, 2) - 128, 0, Q0 + VH))

        two = (e >= C0) & (e < C0 + 2 * (Q0 + VH)) & (_mod(e - C0, 2) == 1)

        def chunk(j):
            for a in range(2):
                pl.when(_div(done + j, NU) == a)(lambda: attend(a, done + j - a * NU))

        _loop(jnp.where(s >= 0, _div(w, 8), jnp.where(e < 0, 0, jnp.where(two, 2, 1))), chunk)

        @pl.when((w > 0) & (w < 8))
        def _():
            wait_all(wo_v.at[w], s_o.at[w])
            o_proj(w)

    _loop(steps + len(tail), step)

    part = jnp.where(jax.lax.broadcasted_iota(jnp.int32, (8, D), 0) == 0, y_v[1], 0.0)
    gate = y_v[0]
    x = jnp.broadcast_to(x_v[0].astype(F32), (8, D))
    for i in VPU_ORDER:
        rows = _ds(i, 16)
        wait_all(wo_v.at[0, :, rows, :], s_o.at[8 + i])
        for j in range(4):
            prod = wo_v[0, j, rows, :].astype(F32) * jnp.concatenate([c_v[j, rows, :]] * (D // DH), axis=1)
            part = part + (prod[0:8] + prod[8:16])
    res = x + jnp.broadcast_to(jnp.sum(part, axis=0, keepdims=True), (8, D)) * gate
    out_ref[0] = res.astype(out_ref.dtype)[0:1]


@jax.jit
def pallas_recurrent_scan__sliding_block_cached__moe_arch_mod__decode_kernel(
    A_x: jax.Array,
    A_k_cache: jax.Array,
    A_v_cache: jax.Array,
    A_wq: jax.Array,
    A_wo: jax.Array,
    B_x: jax.Array,
    B_w_r: jax.Array,
    B_w_gate: jax.Array,
    B_w_up: jax.Array,
    B_w_down: jax.Array,
):
    del B_x
    hbm = pl.BlockSpec(memory_space=pltpu.HBM)
    dma = pltpu.SemaphoreType.DMA
    return pl.pallas_call(
        _kernel,
        out_shape=jax.ShapeDtypeStruct((1, 1, D), BF16),
        in_specs=[hbm] * 9,
        out_specs=pl.BlockSpec(memory_space=pltpu.VMEM),
        scratch_shapes=[
            pltpu.VMEM((1, 1, D), BF16),
            pltpu.VMEM((D,), BF16),
            pltpu.VMEM((4, 4, D // 4, 1024), BF16),
            pltpu.VMEM((2, NH, W, DH), BF16),
            pltpu.VMEM((8, 4, DH, D), BF16),
            pltpu.VMEM((3, F, D), BF16),
            pltpu.VMEM((8, D), F32),
            pltpu.VMEM((NH, DH), F32),
            pltpu.VMEM((NC, CK // 128, NH, 128), F32),
            pltpu.VMEM((NH, 128), F32),
            pltpu.VMEM((NH, 128), F32),
            pltpu.VMEM((NH, DH), F32),
            pltpu.VMEM((2, 8, D), F32),
            pltpu.VMEM((4, DH, DH), F32),
            dma((2,)), dma((4,)), dma((2 * NU,)), dma((1,)), dma((16,)),
        ],
        compiler_params=pltpu.CompilerParams(
            vmem_limit_bytes=100 * 1024 * 1024,
            disable_bounds_checks=True,
            disable_semaphore_checks=True,
        ),
    )(A_x, A_k_cache, A_v_cache, A_wq.reshape(4, D // 4, NH * DH), A_wo.reshape(4, 8, DH, D), B_w_r,
      B_w_gate.T.reshape(2, F // 2, D), B_w_up.T.reshape(2, F // 2, D), B_w_down.reshape(2, F // 2, D))
```
